```python
import jax
import jax.numpy as jnp

def _softmax(x, axis=-1):
    return jax.nn.softmax(x, axis=axis)
def _gelu(x):
    return jax.nn.gelu(x, approximate=True)
def _silu(x):
    return jax.nn.silu(x)
def _sigmoid(x):
    return jax.nn.sigmoid(x)
def _layernorm(x, axis=-1, eps=1e-5):
    m = jnp.mean(x, axis=axis, keepdims=True)
    v = jnp.var(x, axis=axis, keepdims=True)
    return (x - m) / jnp.sqrt(v + eps)
def _scatter_add(tgt, idx, src, axis=0):
    return tgt.at[idx].add(src)
def _segment_sum(src, seg, n):
    return jax.ops.segment_sum(src, seg, n)
class _Rng:
    def __init__(self, key):
        self._k = key
    def _next(self):
        self._k, sub = jax.random.split(self._k)
        return sub
    def normal(self, shape):
        return jax.random.normal(self._next(), shape, dtype=jnp.bfloat16)
    def randint(self, lo, hi, shape):
        return jax.random.randint(self._next(), shape, lo, hi, dtype=jnp.int32)
    def uniform(self, shape, lo=0.0, hi=1.0):
        return jax.random.uniform(self._next(), shape, jnp.bfloat16, lo, hi)
    def permutation(self, n):
        return jax.random.permutation(self._next(), n)


kernel_name = 'gated_mix__sliding_block_cached__glu_gated_swiglu__decode'

def setup_inputs():
    _rng = _Rng(jax.random.key(int.from_bytes(__import__("os").urandom(4), "little")))
    _w = (lambda a: (lambda t: t.astype(jnp.bfloat16) if jnp.issubdtype(t.dtype, jnp.floating) else t)(jnp.asarray(a)))
    def _A_setup():
        B, Sq, D = 1, 1, 640
        Hq, Hkv, Sk, Dh = 32, 32, 32768, 192
        assert Hq % Hkv == 0, (Hq, Hkv)
        return {
            "x": _w((lambda *s: _rng.normal(s) * 0.05)(B, Sq, D)),
            "k_cache": _w((lambda *s: _rng.normal(s) * 0.05)(B, Hkv, Sk, Dh)),
            "v_cache": _w((lambda *s: _rng.normal(s) * 0.05)(B, Hkv, Sk, Dh)),
            "wq": _w((lambda *s: _rng.normal(s) * 0.05)(D, Hq * Dh) * (D ** -0.5)),
            "wo": _w((lambda *s: _rng.normal(s) * 0.05)(Hq * Dh, D) * ((Hq * Dh) ** -0.5)),
        }
    _A_in = _A_setup()

    def _B_setup():
        B, S, D, F = 1, 1, 640, 1536
        return {
            "x": _w((lambda *s: _rng.normal(s) * 0.05)(B, S, D)),
            "w1": _w((lambda *s: _rng.normal(s) * 0.05)(D, F) * (2.0 / D) ** 0.5),
            "w3": _w((lambda *s: _rng.normal(s) * 0.05)(D, F) * (2.0 / D) ** 0.5),
            "w2": _w((lambda *s: _rng.normal(s) * 0.05)(F, D) * (2.0 / F) ** 0.5),
        }
    _B_in = _B_setup()

    return {
        "A_x": _A_in["x"],
        "A_k_cache": _A_in["k_cache"],
        "A_v_cache": _A_in["v_cache"],
        "A_wq": _A_in["wq"],
        "A_wo": _A_in["wo"],
        "B_x": _B_in["x"],
        "B_w1": _B_in["w1"],
        "B_w3": _B_in["w3"],
        "B_w2": _B_in["w2"],
        "gate_w": _w((lambda *s: _rng.normal(s) * 0.05)(640)),
    }

def reference(A_x, A_k_cache, A_v_cache, A_wq, A_wo, B_x, B_w1, B_w3, B_w2, gate_w):
    def _A_ref(x, k_cache, v_cache, wq, wo):
        B, Sq, D = x.shape
        Hq, Dh = 32, 192
        Hkv, Sk = k_cache.shape[1], k_cache.shape[2]
        W = min(4096, max(256, Sk // 4))
        rep = Hq // Hkv
        q = (lambda x, *d: x.transpose(*d))((x @ wq).reshape(B, Sq, Hq, Dh), 0, 2, 1, 3)
        k = jnp.repeat(k_cache[:, :, Sk - W:, :], rep, axis=1)
        v = jnp.repeat(v_cache[:, :, Sk - W:, :], rep, axis=1)
        scores = jnp.einsum("bhqd,bhkd->bhqk", q, k) * (Dh ** -0.5)
        p = _softmax(scores, axis=-1)
        o = jnp.einsum("bhqk,bhkd->bhqd", p, v)
        return (lambda x, *d: x.transpose(*d))(o, 0, 2, 1, 3).reshape(B, Sq, Hq * Dh) @ wo

    def _B_ref(x, w1, w3, w2):
        gate = jnp.einsum("bsd,df->bsf", x, w1)
        up = jnp.einsum("bsd,df->bsf", x, w3)
        h = _silu(gate) * up
        out = jnp.einsum("bsf,fd->bsd", h, w2)
        return out

    x = A_x
    g = _sigmoid((x * gate_w).sum(-1, keepdims=True))
    a = _A_ref(x, A_k_cache, A_v_cache, A_wq, A_wo)
    b = _B_ref(x, B_w1, B_w3, B_w2)
    return g * a + (1 - g) * b
```

```python
import functools

import jax
import jax.numpy as jnp
from jax import lax
from jax.experimental import pallas as pl
from jax.experimental.pallas import tpu as pltpu

LANES = 128
NSLOT = 64
DEPTH = 32
P1_ROWS = 160


def _col_bcast(row):
    n = row.shape[1]
    return jnp.broadcast_to(row, (LANES, n)).T


def _kernel(x_hbm, kt_hbm, vt_hbm, wq_hbm, wo_hbm, w1_hbm, w3_hbm, w2_hbm, gw_hbm,
            out_ref,
            ring, xv, gv, xb_ref, qb_ref, cb_ref, s_ref, sems, small_sems,
            *, n_heads, dh, seq, win, d_model, d_ff):
    f32 = jnp.float32
    half = dh // 2
    n_ct = win // LANES
    assert n_ct == DEPTH and NSLOT == 2 * DEPTH
    n_sub = d_model // P1_ROWS
    n_q = (n_heads * dh) // LANES
    n_f = d_ff // LANES
    n_oc = d_model // LANES
    nb_f = d_ff // dh
    nb = nb_f + n_heads
    col0 = seq - win
    scale = float(dh) ** -0.5

    def start_tile(src, r0, c0, rows, slot):
        hr = rows // 2
        for part in range(2):
            pltpu.make_async_copy(
                src.at[pl.ds(r0 + part * hr, hr), pl.ds(c0, LANES)],
                ring.at[slot, pl.ds(part * hr, hr), :],
                sems.at[slot],
            ).start(priority=part)

    def wait_tile(rows, slot):
        view = ring.at[slot, pl.ds(0, rows), :]
        pltpu.make_async_copy(view, view, sems.at[slot]).wait()

    def mult(v, m):
        return v if isinstance(v, int) else pl.multiple_of(v, m)

    def start_p1(src, j, u, slot):
        start_tile(src, u * P1_ROWS, mult(j * LANES, LANES), P1_ROWS, slot)

    def start_kv(src, h, c, slot):
        start_tile(src.at[0, h], 0, mult(col0 + c * LANES, LANES), dh, slot)

    def start_p3(src, b, cj, slot):
        start_tile(src, mult(b * dh, dh), mult(cj * LANES, LANES), dh, slot)

    x_cp = pltpu.make_async_copy(x_hbm, xv, small_sems.at[0])
    g_cp = pltpu.make_async_copy(gw_hbm, gv, small_sems.at[1])
    x_cp.start()
    g_cp.start()
    for i in range(DEPTH):
        sl, u = divmod(i, n_sub)
        start_p1((w1_hbm, w3_hbm)[sl % 2], sl // 2, u, i)

    x_cp.wait()
    g_cp.wait()
    x = xv[0].astype(f32)
    gw = gv[...].astype(f32)
    gacc = x[:, 0:LANES] * gw[0:1, :]
    for r in range(1, n_oc):
        gacc = gacc + x[:, r * LANES:(r + 1) * LANES] * gw[r:r + 1, :]
    g = jax.nn.sigmoid(jnp.sum(gacc, axis=1, keepdims=True))
    xb_ref[...] = _col_bcast(x)

    def p1_slice(step0, issue):
        acc = None
        for u in range(n_sub):
            slot = (step0 + u) % NSLOT
            wait_tile(P1_ROWS, slot)
            issue(u, (slot + DEPTH) % NSLOT)
            t = ring[slot, pl.ds(0, P1_ROWS), :].astype(f32)
            prod = t * xb_ref[pl.ds(u * P1_ROWS, P1_ROWS), :]
            part = jnp.sum(prod.reshape(P1_ROWS // 8, 8, LANES), axis=0)
            acc = part if acc is None else acc + part
        return jnp.sum(acc, axis=0, keepdims=True)

    sl_ahead = DEPTH // n_sub
    f_ahead = sl_ahead // 2

    def ffn_body(f, carry, *, tail):
        step0 = f * (2 * n_sub)
        if tail:
            j = 2 * (f - (n_f - f_ahead))
            iss_a = lambda u, s: start_p1(wq_hbm, j, u, s)
            iss_b = lambda u, s: start_p1(wq_hbm, j + 1, u, s)
        else:
            iss_a = lambda u, s: start_p1(w1_hbm, f + f_ahead, u, s)
            iss_b = lambda u, s: start_p1(w3_hbm, f + f_ahead, u, s)
        gate = p1_slice(step0, iss_a)
        up = p1_slice(step0 + n_sub, iss_b)
        hid = (gate * jax.nn.sigmoid(gate)) * up * (1.0 - g)
        cb_ref[pl.ds(pl.multiple_of(f * LANES, LANES), LANES), :] = _col_bcast(hid)
        return carry

    lax.fori_loop(0, n_f - f_ahead, functools.partial(ffn_body, tail=False), 0)
    lax.fori_loop(n_f - f_ahead, n_f, functools.partial(ffn_body, tail=True), 0)

    p1_ffn_steps = 2 * n_f * n_sub

    def q_body(j, carry, *, tail):
        step0 = p1_ffn_steps + j * n_sub
        if tail:
            c0 = (j - (n_q - sl_ahead)) * n_sub
            iss = lambda u, s: start_kv(kt_hbm, 0, c0 + u, s)
        else:
            iss = lambda u, s: start_p1(wq_hbm, j + sl_ahead, u, s)
        q = p1_slice(step0, iss) * scale
        qb_ref[pl.ds(pl.multiple_of(j * LANES, LANES), LANES), :] = _col_bcast(q)
        return carry

    lax.fori_loop(0, n_q - sl_ahead, functools.partial(q_body, tail=False), 0)
    lax.fori_loop(n_q - sl_ahead, n_q, functools.partial(q_body, tail=True), 0)

    p1_steps = p1_ffn_steps + n_q * n_sub
    k_base = p1_steps % NSLOT
    v_base = (k_base + DEPTH) % NSLOT
    assert k_base % DEPTH == 0

    def head_body(h, carry, *, last):
        qb = qb_ref[pl.ds(mult(h * dh, dh), dh), :]

        def k_step(c, carry):
            wait_tile(dh, k_base + c)
            start_kv(vt_hbm, h, c, v_base + c)
            t = ring[k_base + c].astype(f32)
            s_ref[pl.ds(c, 1), :] = jnp.sum(t * qb, axis=0, keepdims=True)
            return carry

        lax.fori_loop(0, n_ct, k_step, 0)

        s = s_ref[...]
        m = jnp.max(jnp.max(s, axis=0, keepdims=True), axis=1, keepdims=True)
        p = jnp.exp(s - m)
        l = jnp.sum(jnp.sum(p, axis=0, keepdims=True), axis=1, keepdims=True)
        s_ref[...] = p

        def v_step(c, acc):
            wait_tile(dh, v_base + c)
            if last:
                start_p3(w2_hbm, lax.div(c, n_oc), lax.rem(c, n_oc), k_base + c)
            else:
                start_kv(kt_hbm, h + 1, c, k_base + c)
            t = ring[v_base + c].astype(f32)
            return acc + t * s_ref[pl.ds(c, 1), :]

        acc = lax.fori_loop(0, n_ct, v_step, jnp.zeros((dh, LANES), f32))
        o = jnp.sum(acc, axis=1, keepdims=True) * (g / l)
        cb_ref[pl.ds(mult(d_ff + h * dh, dh), dh), :] = jnp.broadcast_to(o, (dh, LANES))
        return carry

    lax.fori_loop(0, n_heads - 1, functools.partial(head_body, last=False), 0)
    head_body(n_heads - 1, 0, last=True)

    b_ahead, c_ahead = divmod(DEPTH, n_oc)
    assert b_ahead + 1 < nb_f + 1

    def p3_body(b, acc, *, mode):
        cb = cb_ref[pl.ds(mult(b * dh, dh), dh), :]
        new = []
        for cj in range(n_oc):
            slot = (k_base + b * n_oc + cj) % NSLOT
            wait_tile(dh, slot)
            nc = cj + c_ahead
            tb = b + b_ahead + nc // n_oc
            nslot = (slot + DEPTH) % NSLOT
            if mode == "static":
                if tb < nb_f:
                    start_p3(w2_hbm, tb, nc % n_oc, nslot)
                elif tb < nb:
                    start_p3(wo_hbm, tb - nb_f, nc % n_oc, nslot)
            elif mode == "wo":
                start_p3(wo_hbm, tb - nb_f, nc % n_oc, nslot)
            t = ring[slot].astype(f32)
            part = jnp.sum((t * cb).reshape(dh // 8, 8, LANES), axis=0)
            new.append(acc[cj] + part)
        return tuple(new)

    acc = tuple(jnp.zeros((8, LANES), f32) for _ in range(n_oc))
    b_lo = nb_f - b_ahead
    b_hi = nb - b_ahead - 1
    for b in range(b_lo):
        acc = p3_body(b, acc, mode="static")
    acc = lax.fori_loop(b_lo, b_hi, functools.partial(p3_body, mode="wo"), acc)
    acc = p3_body(b_hi, acc, mode="static")
    acc = lax.fori_loop(b_hi + 1, nb, functools.partial(p3_body, mode="none"), acc)

    res = jnp.concatenate([jnp.sum(a, axis=0, keepdims=True) for a in acc], axis=1)
    out_ref[0] = res.astype(out_ref.dtype)


@jax.jit
def pallas_gated_mix__sliding_block_cached__glu_gated_swiglu__decode_kernel(
    A_x: jax.Array,
    A_k_cache: jax.Array,
    A_v_cache: jax.Array,
    A_wq: jax.Array,
    A_wo: jax.Array,
    B_x: jax.Array,
    B_w1: jax.Array,
    B_w3: jax.Array,
    B_w2: jax.Array,
    gate_w: jax.Array,
):
    del B_x
    _, _, d_model = A_x.shape
    _, n_heads, seq, dh = A_k_cache.shape
    d_ff = B_w1.shape[1]
    win = min(4096, max(256, seq // 4))

    kt = jnp.swapaxes(A_k_cache, 2, 3)
    vt = jnp.swapaxes(A_v_cache, 2, 3)
    gw = gate_w.reshape(d_model // LANES, LANES)

    kernel = functools.partial(
        _kernel, n_heads=n_heads, dh=dh, seq=seq, win=win, d_model=d_model, d_ff=d_ff)
    return pl.pallas_call(
        kernel,
        out_shape=jax.ShapeDtypeStruct(A_x.shape, A_x.dtype),
        in_specs=[pl.BlockSpec(memory_space=pl.ANY)] * 9,
        out_specs=pl.BlockSpec(memory_space=pltpu.VMEM),
        scratch_shapes=[
            pltpu.VMEM((NSLOT, dh, LANES), jnp.bfloat16),
            pltpu.VMEM(A_x.shape, jnp.bfloat16),
            pltpu.VMEM(gw.shape, jnp.bfloat16),
            pltpu.VMEM((d_model, LANES), jnp.float32),
            pltpu.VMEM((n_heads * dh, LANES), jnp.float32),
            pltpu.VMEM((d_ff + n_heads * dh, LANES), jnp.float32),
            pltpu.VMEM((win // LANES, LANES), jnp.float32),
            pltpu.SemaphoreType.DMA((NSLOT,)),
            pltpu.SemaphoreType.DMA((2,)),
        ],
        compiler_params=pltpu.CompilerParams(
            vmem_limit_bytes=32 * 1024 * 1024,
            disable_bounds_checks=True,
        ),
    )(A_x, kt, vt, A_wq, A_wo, B_w1, B_w3, B_w2, gw)
```

```python
import functools

import jax
import jax.numpy as jnp
from jax import lax
from jax.experimental import pallas as pl
from jax.experimental.pallas import tpu as pltpu

LANES = 128
NSLOT = 64
DEPTH = 32
P1_ROWS = 160


def _col_bcast(row):
    n = row.shape[1]
    return jnp.broadcast_to(row, (LANES, n)).T


def _bcast_group(row, off, n):
    lane = lax.broadcasted_iota(jnp.int32, (n, LANES), 1)
    idx = lax.broadcasted_iota(jnp.int32, (n, LANES), 0)
    picked = jnp.where(lane - idx == off, row, 0.0)
    return jnp.broadcast_to(jnp.sum(picked, axis=1, keepdims=True), (n, LANES))


def _fold8(v):
    parts = [v[i:i + 8] for i in range(0, v.shape[0], 8)]
    while len(parts) > 1:
        nxt = [parts[i] + parts[i + 1] for i in range(0, len(parts) - 1, 2)]
        if len(parts) % 2:
            nxt.append(parts[-1])
        parts = nxt
    return parts[0]


def _kernel(x_hbm, kt_hbm, vt_hbm, wq_hbm, wo_hbm, w1_hbm, w3_hbm, w2_hbm, gw_hbm,
            out_ref,
            ring, xv, gv, xb_ref, q_ref, h_ref, qb_ref, cb_ref, s_ref, sems,
            *, n_heads, dh, seq, win, d_model, d_ff):
    f32 = jnp.float32
    half = dh // 2
    n_ct = win // LANES
    assert n_ct == DEPTH and NSLOT == 2 * DEPTH
    n_sub = d_model // P1_ROWS
    n_q = (n_heads * dh) // LANES
    n_f = d_ff // LANES
    n_oc = d_model // LANES
    nb_f = d_ff // dh
    nb = nb_f + n_heads
    col0 = seq - win
    scale = float(dh) ** -0.5

    def start_tile(src, r0, c0, rows, slot):
        hr = rows // 2
        for part in range(2):
            pltpu.make_async_copy(
                src.at[pl.ds(r0 + part * hr, hr), pl.ds(c0, LANES)],
                ring.at[slot, pl.ds(part * hr, hr), :],
                sems.at[slot],
            ).start(priority=part)

    def wait_tile(rows, slot):
        view = ring.at[slot, pl.ds(0, rows), :]
        pltpu.make_async_copy(view, view, sems.at[slot]).wait()

    def wrap(slot):
        return slot % NSLOT if isinstance(slot, int) else slot & (NSLOT - 1)

    def mult(v, m):
        return v if isinstance(v, int) else pl.multiple_of(v, m)

    def start_p1(src, j, u, slot):
        start_tile(src, u * P1_ROWS, mult(j * LANES, LANES), P1_ROWS, slot)

    def start_kv(src, h, c, slot):
        start_tile(src.at[0, h], 0, mult(col0 + c * LANES, LANES), dh, slot)

    def start_p3(src, b, cj, slot):
        start_tile(src, mult(b * dh, dh), mult(cj * LANES, LANES), dh, slot)

    x_cp = pltpu.make_async_copy(x_hbm, xv, sems.at[NSLOT])
    g_cp = pltpu.make_async_copy(gw_hbm, gv, sems.at[NSLOT + 1])
    x_cp.start()
    g_cp.start()
    for i in range(DEPTH):
        sl, u = divmod(i, n_sub)
        start_p1((w1_hbm, w3_hbm)[sl % 2], sl // 2, u, i)

    x_cp.wait()
    g_cp.wait()
    x = xv[0].astype(f32)
    gw = gv[...].astype(f32)
    gacc = x[:, 0:LANES] * gw[0:1, :]
    for r in range(1, n_oc):
        gacc = gacc + x[:, r * LANES:(r + 1) * LANES] * gw[r:r + 1, :]
    g = jax.nn.sigmoid(jnp.sum(gacc, axis=1, keepdims=True))
    xb_ref[...] = _col_bcast(x)

    def p1_slice(step0, issue):
        acc = None
        for u in range(n_sub):
            slot = wrap(step0 + u)
            wait_tile(P1_ROWS, slot)
            issue(u, wrap(step0 + u + DEPTH))
            t = ring[slot, pl.ds(0, P1_ROWS), :].astype(f32)
            prod = t * xb_ref[pl.ds(u * P1_ROWS, P1_ROWS), :]
            part = _fold8(prod)
            acc = part if acc is None else acc + part
        return jnp.sum(acc, axis=0, keepdims=True)

    sl_ahead = DEPTH // n_sub
    f_ahead = sl_ahead // 2

    def ffn_body(f, carry, *, tail):
        step0 = f * (2 * n_sub)
        if tail:
            j = 2 * (f - (n_f - f_ahead))
            iss_a = lambda u, s: start_p1(wq_hbm, j, u, s)
            iss_b = lambda u, s: start_p1(wq_hbm, j + 1, u, s)
        else:
            iss_a = lambda u, s: start_p1(w1_hbm, f + f_ahead, u, s)
            iss_b = lambda u, s: start_p1(w3_hbm, f + f_ahead, u, s)
        gate = p1_slice(step0, iss_a)
        up = p1_slice(step0 + n_sub, iss_b)
        hid = (gate * jax.nn.sigmoid(gate)) * up * (1.0 - g)
        h_ref[pl.ds(f, 1), :] = hid
        return carry

    with jax.named_scope("p1_ffn"):
        lax.fori_loop(0, n_f - f_ahead, functools.partial(ffn_body, tail=False), 0)
        lax.fori_loop(n_f - f_ahead, n_f, functools.partial(ffn_body, tail=True), 0)

    p1_ffn_steps = 2 * n_f * n_sub

    def q_body(j, carry, *, tail):
        step0 = p1_ffn_steps + j * n_sub
        if tail:
            c0 = (j - (n_q - sl_ahead)) * n_sub
            iss = lambda u, s: start_kv(kt_hbm, 0, c0 + u, s)
        else:
            iss = lambda u, s: start_p1(wq_hbm, j + sl_ahead, u, s)
        q = p1_slice(step0, iss) * scale
        q_ref[pl.ds(j, 1), :] = q
        return carry

    with jax.named_scope("p1_q"):
        lax.fori_loop(0, n_q - sl_ahead, functools.partial(q_body, tail=False), 0)
        lax.fori_loop(n_q - sl_ahead, n_q, functools.partial(q_body, tail=True), 0)

    p1_steps = p1_ffn_steps + n_q * n_sub
    k_base = p1_steps % NSLOT
    v_base = (k_base + DEPTH) % NSLOT
    assert k_base % DEPTH == 0

    hg = LANES // 2
    assert dh == 3 * hg and d_ff == n_heads * 48

    def make_qb(h):
        r0 = (3 * h) >> 1
        par = h & 1
        for gi, (r, off) in enumerate(
                ((r0, par * hg), (r0 + par, (1 - par) * hg), (r0 + 1, par * hg))):
            qb_ref[pl.ds(gi * hg, hg), :] = _bcast_group(q_ref[pl.ds(r, 1), :], off, hg)

    def make_hb(h):
        for t in range(3):
            e = h * 48 + t * 16
            cb_ref[pl.ds(mult(e, 16), 16), :] = _bcast_group(
                h_ref[pl.ds(e >> 7, 1), :], e & (LANES - 1), 16)

    make_qb(0)

    def head_body(h, carry, *, last):
        qb = qb_ref[...]

        def k_step(c, carry):
            wait_tile(dh, k_base + c)
            start_kv(vt_hbm, h, c, v_base + c)
            t = ring[k_base + c].astype(f32)
            s_ref[pl.ds(c, 1), :] = jnp.sum(_fold8(t * qb), axis=0, keepdims=True)
            return carry

        lax.fori_loop(0, n_ct, k_step, 0)

        s = s_ref[...]
        m = jnp.max(jnp.max(s, axis=0, keepdims=True), axis=1, keepdims=True)
        p = jnp.exp(s - m)
        l_row = jnp.sum(p, axis=0, keepdims=True)
        s_ref[...] = p
        if not last:
            make_qb(h + 1)
        make_hb(h)

        def v_step(c, acc):
            wait_tile(dh, v_base + c)
            if last:
                start_p3(w2_hbm, lax.div(c, n_oc), lax.rem(c, n_oc), k_base + c)
            else:
                start_kv(kt_hbm, h + 1, c, k_base + c)
            t = ring[v_base + c].astype(f32)
            return acc + t * s_ref[pl.ds(c, 1), :]

        acc = lax.fori_loop(0, n_ct, v_step, jnp.zeros((dh, LANES), f32))
        l = jnp.sum(l_row, axis=1, keepdims=True)
        o = jnp.sum(acc, axis=1, keepdims=True) * (g / l)
        cb_ref[pl.ds(mult(d_ff + h * dh, dh), dh), :] = jnp.broadcast_to(o, (dh, LANES))
        return carry

    with jax.named_scope("p2"):
        lax.fori_loop(0, n_heads - 1, functools.partial(head_body, last=False), 0)
        head_body(n_heads - 1, 0, last=True)

    b_ahead, c_ahead = divmod(DEPTH, n_oc)
    assert b_ahead + 1 < nb_f + 1

    def p3_body(b, acc, *, mode):
        cb = cb_ref[pl.ds(mult(b * dh, dh), dh), :]
        new = []
        for cj in range(n_oc):
            slot = wrap(k_base + b * n_oc + cj)
            wait_tile(dh, slot)
            nc = cj + c_ahead
            tb = b + b_ahead + nc // n_oc
            nslot = wrap(k_base + b * n_oc + cj + DEPTH)
            if mode == "static":
                if tb < nb_f:
                    start_p3(w2_hbm, tb, nc % n_oc, nslot)
                elif tb < nb:
                    start_p3(wo_hbm, tb - nb_f, nc % n_oc, nslot)
            elif mode == "wo":
                start_p3(wo_hbm, tb - nb_f, nc % n_oc, nslot)
            t = ring[slot].astype(f32)
            part = _fold8(t * cb)
            new.append(acc[cj] + part)
        return tuple(new)

    acc = tuple(jnp.zeros((8, LANES), f32) for _ in range(n_oc))
    b_lo = nb_f - b_ahead
    b_hi = nb - b_ahead - 1
    with jax.named_scope("p3"):
        for b in range(b_lo):
            acc = p3_body(b, acc, mode="static")
        acc = lax.fori_loop(b_lo, b_hi, functools.partial(p3_body, mode="wo"), acc)
        acc = p3_body(b_hi, acc, mode="static")
        acc = lax.fori_loop(b_hi + 1, nb, functools.partial(p3_body, mode="none"), acc)

    res = jnp.concatenate([jnp.sum(a, axis=0, keepdims=True) for a in acc], axis=1)
    out_ref[0] = res.astype(out_ref.dtype)


@jax.jit
def pallas_gated_mix__sliding_block_cached__glu_gated_swiglu__decode_kernel(
    A_x: jax.Array,
    A_k_cache: jax.Array,
    A_v_cache: jax.Array,
    A_wq: jax.Array,
    A_wo: jax.Array,
    B_x: jax.Array,
    B_w1: jax.Array,
    B_w3: jax.Array,
    B_w2: jax.Array,
    gate_w: jax.Array,
):
    del B_x
    _, _, d_model = A_x.shape
    _, n_heads, seq, dh = A_k_cache.shape
    d_ff = B_w1.shape[1]
    win = min(4096, max(256, seq // 4))

    kt = jnp.swapaxes(A_k_cache, 2, 3)
    vt = jnp.swapaxes(A_v_cache, 2, 3)
    gw = gate_w.reshape(d_model // LANES, LANES)

    kernel = functools.partial(
        _kernel, n_heads=n_heads, dh=dh, seq=seq, win=win, d_model=d_model, d_ff=d_ff)
    return pl.pallas_call(
        kernel,
        out_shape=jax.ShapeDtypeStruct(A_x.shape, A_x.dtype),
        in_specs=[pl.BlockSpec(memory_space=pl.ANY)] * 9,
        out_specs=pl.BlockSpec(memory_space=pltpu.VMEM),
        scratch_shapes=[
            pltpu.VMEM((NSLOT, dh, LANES), jnp.bfloat16),
            pltpu.VMEM(A_x.shape, jnp.bfloat16),
            pltpu.VMEM(gw.shape, jnp.bfloat16),
            pltpu.VMEM((d_model, LANES), jnp.float32),
            pltpu.VMEM((n_heads * dh // LANES, LANES), jnp.float32),
            pltpu.VMEM((d_ff // LANES, LANES), jnp.float32),
            pltpu.VMEM((dh, LANES), jnp.float32),
            pltpu.VMEM((d_ff + n_heads * dh, LANES), jnp.float32),
            pltpu.VMEM((win // LANES, LANES), jnp.float32),
            pltpu.SemaphoreType.DMA((NSLOT + 2,)),
        ],
        compiler_params=pltpu.CompilerParams(
            vmem_limit_bytes=32 * 1024 * 1024,
            disable_bounds_checks=True,
        ),
    )(A_x, kt, vt, A_wq, A_wo, B_w1, B_w3, B_w2, gw)
```

```python
import functools

import jax
import jax.numpy as jnp
from jax import lax
from jax.experimental import pallas as pl
from jax.experimental.pallas import tpu as pltpu

LANES = 128
NSLOT = 64
DEPTH = 32
HI_ROWS = 16
P1_ROWS = 160


def _col_bcast(row):
    n = row.shape[1]
    return jnp.broadcast_to(row, (LANES, n)).T


def _bcast_group(row, off, n):
    lane = lax.broadcasted_iota(jnp.int32, (n, LANES), 1)
    idx = lax.broadcasted_iota(jnp.int32, (n, LANES), 0)
    picked = jnp.where(lane - idx == off, row, 0.0)
    return jnp.broadcast_to(jnp.sum(picked, axis=1, keepdims=True), (n, LANES))


def _fold8(v):
    parts = [v[i:i + 8] for i in range(0, v.shape[0], 8)]
    while len(parts) > 1:
        nxt = [parts[i] + parts[i + 1] for i in range(0, len(parts) - 1, 2)]
        if len(parts) % 2:
            nxt.append(parts[-1])
        parts = nxt
    return parts[0]


def _kernel(x_hbm, kt_hbm, vt_hbm, wq_hbm, wo_hbm, w1_hbm, w3_hbm, w2_hbm, gw_hbm,
            out_ref,
            ring, xv, gv, xb_ref, q_ref, h_ref, qb_ref, cb_ref, s_ref, sems,
            *, n_heads, dh, seq, win, d_model, d_ff):
    f32 = jnp.float32
    half = dh // 2
    n_ct = win // LANES
    assert n_ct == DEPTH and NSLOT == 2 * DEPTH
    n_sub = d_model // P1_ROWS
    n_q = (n_heads * dh) // LANES
    n_f = d_ff // LANES
    n_oc = d_model // LANES
    nb_f = d_ff // dh
    nb = nb_f + n_heads
    col0 = seq - win
    scale = float(dh) ** -0.5

    def start_tile(src, r0, c0, rows, slot):
        for part, (o, n) in enumerate(((0, HI_ROWS), (HI_ROWS, rows - HI_ROWS))):
            pltpu.make_async_copy(
                src.at[pl.ds(r0 + o, n), pl.ds(c0, LANES)],
                ring.at[slot, pl.ds(o, n), :],
                sems.at[slot],
            ).start(priority=part)

    def wait_tile(rows, slot):
        view = ring.at[slot, pl.ds(0, rows), :]
        pltpu.make_async_copy(view, view, sems.at[slot]).wait()

    def wrap(slot):
        return slot % NSLOT if isinstance(slot, int) else slot & (NSLOT - 1)

    def mult(v, m):
        return v if isinstance(v, int) else pl.multiple_of(v, m)

    def start_p1(src, j, u, slot):
        start_tile(src, u * P1_ROWS, mult(j * LANES, LANES), P1_ROWS, slot)

    def start_kv(src, h, c, slot):
        start_tile(src.at[0, h], 0, mult(col0 + c * LANES, LANES), dh, slot)

    def start_p3(src, b, cj, slot):
        start_tile(src, mult(b * dh, dh), mult(cj * LANES, LANES), dh, slot)

    x_cp = pltpu.make_async_copy(x_hbm, xv, sems.at[NSLOT])
    g_cp = pltpu.make_async_copy(gw_hbm, gv, sems.at[NSLOT + 1])
    x_cp.start()
    g_cp.start()
    for i in range(DEPTH):
        sl, u = divmod(i, n_sub)
        start_p1((w1_hbm, w3_hbm)[sl % 2], sl // 2, u, i)

    x_cp.wait()
    g_cp.wait()
    x = xv[0].astype(f32)
    gw = gv[...].astype(f32)
    gacc = x[:, 0:LANES] * gw[0:1, :]
    for r in range(1, n_oc):
        gacc = gacc + x[:, r * LANES:(r + 1) * LANES] * gw[r:r + 1, :]
    g = jax.nn.sigmoid(jnp.sum(gacc, axis=1, keepdims=True))
    xb_ref[...] = _col_bcast(x)

    def p1_slice(step0, issue):
        acc = None
        for u in range(n_sub):
            slot = wrap(step0 + u)
            wait_tile(P1_ROWS, slot)
            issue(u, wrap(step0 + u + DEPTH))
            t = ring[slot, pl.ds(0, P1_ROWS), :].astype(f32)
            prod = t * xb_ref[pl.ds(u * P1_ROWS, P1_ROWS), :]
            part = _fold8(prod)
            acc = part if acc is None else acc + part
        return jnp.sum(acc, axis=0, keepdims=True)

    sl_ahead = DEPTH // n_sub
    f_ahead = sl_ahead // 2

    def ffn_body(f, carry, *, tail):
        step0 = f * (2 * n_sub)
        if tail:
            j = 2 * (f - (n_f - f_ahead))
            iss_a = lambda u, s: start_p1(wq_hbm, j, u, s)
            iss_b = lambda u, s: start_p1(wq_hbm, j + 1, u, s)
        else:
            iss_a = lambda u, s: start_p1(w1_hbm, f + f_ahead, u, s)
            iss_b = lambda u, s: start_p1(w3_hbm, f + f_ahead, u, s)
        gate = p1_slice(step0, iss_a)
        up = p1_slice(step0 + n_sub, iss_b)
        hid = (gate * jax.nn.sigmoid(gate)) * up * (1.0 - g)
        h_ref[pl.ds(f, 1), :] = hid
        return carry

    with jax.named_scope("p1_ffn"):
        lax.fori_loop(0, n_f - f_ahead, functools.partial(ffn_body, tail=False), 0)
        lax.fori_loop(n_f - f_ahead, n_f, functools.partial(ffn_body, tail=True), 0)

    p1_ffn_steps = 2 * n_f * n_sub

    def q_body(j, carry, *, tail):
        step0 = p1_ffn_steps + j * n_sub
        if tail:
            c0 = (j - (n_q - sl_ahead)) * n_sub
            iss = lambda u, s: start_kv(kt_hbm, 0, c0 + u, s)
        else:
            iss = lambda u, s: start_p1(wq_hbm, j + sl_ahead, u, s)
        q = p1_slice(step0, iss) * scale
        q_ref[pl.ds(j, 1), :] = q
        return carry

    with jax.named_scope("p1_q"):
        lax.fori_loop(0, n_q - sl_ahead, functools.partial(q_body, tail=False), 0)
        lax.fori_loop(n_q - sl_ahead, n_q, functools.partial(q_body, tail=True), 0)

    p1_steps = p1_ffn_steps + n_q * n_sub
    k_base = p1_steps % NSLOT
    v_base = (k_base + DEPTH) % NSLOT
    assert k_base % DEPTH == 0

    hg = LANES // 2
    assert dh == 3 * hg and d_ff == n_heads * 48

    def make_qb(h):
        r0 = (3 * h) >> 1
        par = h & 1
        for gi, (r, off) in enumerate(
                ((r0, par * hg), (r0 + par, (1 - par) * hg), (r0 + 1, par * hg))):
            qb_ref[pl.ds(gi * hg, hg), :] = _bcast_group(q_ref[pl.ds(r, 1), :], off, hg)

    def make_hb(h):
        for t in range(3):
            e = h * 48 + t * 16
            cb_ref[pl.ds(mult(e, 16), 16), :] = _bcast_group(
                h_ref[pl.ds(e >> 7, 1), :], e & (LANES - 1), 16)

    make_qb(0)

    def head_body(h, carry, *, last):
        qb = qb_ref[...]

        def k_step(c, carry):
            wait_tile(dh, k_base + c)
            start_kv(vt_hbm, h, c, v_base + c)
            t = ring[k_base + c].astype(f32)
            s_ref[pl.ds(c, 1), :] = jnp.sum(_fold8(t * qb), axis=0, keepdims=True)
            return carry

        lax.fori_loop(0, n_ct, k_step, 0)

        s = s_ref[...]
        m = jnp.max(jnp.max(s, axis=0, keepdims=True), axis=1, keepdims=True)
        p = jnp.exp(s - m)
        l_row = jnp.sum(p, axis=0, keepdims=True)
        s_ref[...] = p
        if not last:
            make_qb(h + 1)
        make_hb(h)

        def v_step(c, acc):
            wait_tile(dh, v_base + c)
            if last:
                start_p3(w2_hbm, lax.div(c, n_oc), lax.rem(c, n_oc), k_base + c)
            else:
                start_kv(kt_hbm, h + 1, c, k_base + c)
            t = ring[v_base + c].astype(f32)
            return acc + t * s_ref[pl.ds(c, 1), :]

        acc = lax.fori_loop(0, n_ct, v_step, jnp.zeros((dh, LANES), f32))
        l = jnp.sum(l_row, axis=1, keepdims=True)
        o = jnp.sum(acc, axis=1, keepdims=True) * (g / l)
        cb_ref[pl.ds(mult(d_ff + h * dh, dh), dh), :] = jnp.broadcast_to(o, (dh, LANES))
        return carry

    with jax.named_scope("p2"):
        lax.fori_loop(0, n_heads - 1, functools.partial(head_body, last=False), 0)
        head_body(n_heads - 1, 0, last=True)

    b_ahead, c_ahead = divmod(DEPTH, n_oc)
    assert b_ahead + 1 < nb_f + 1

    def p3_body(b, acc, *, mode):
        cb = cb_ref[pl.ds(mult(b * dh, dh), dh), :]
        new = []
        for cj in range(n_oc):
            slot = wrap(k_base + b * n_oc + cj)
            wait_tile(dh, slot)
            nc = cj + c_ahead
            tb = b + b_ahead + nc // n_oc
            nslot = wrap(k_base + b * n_oc + cj + DEPTH)
            if mode == "static":
                if tb < nb_f:
                    start_p3(w2_hbm, tb, nc % n_oc, nslot)
                elif tb < nb:
                    start_p3(wo_hbm, tb - nb_f, nc % n_oc, nslot)
            elif mode == "wo":
                start_p3(wo_hbm, tb - nb_f, nc % n_oc, nslot)
            t = ring[slot].astype(f32)
            part = _fold8(t * cb)
            new.append(acc[cj] + part)
        return tuple(new)

    acc = tuple(jnp.zeros((8, LANES), f32) for _ in range(n_oc))
    b_lo = nb_f - b_ahead
    b_hi = nb - b_ahead - 1
    with jax.named_scope("p3"):
        for b in range(b_lo):
            acc = p3_body(b, acc, mode="static")
        acc = lax.fori_loop(b_lo, b_hi, functools.partial(p3_body, mode="wo"), acc)
        acc = p3_body(b_hi, acc, mode="static")
        acc = lax.fori_loop(b_hi + 1, nb, functools.partial(p3_body, mode="none"), acc)

    res = jnp.concatenate([jnp.sum(a, axis=0, keepdims=True) for a in acc], axis=1)
    out_ref[0] = res.astype(out_ref.dtype)


@jax.jit
def pallas_gated_mix__sliding_block_cached__glu_gated_swiglu__decode_kernel(
    A_x: jax.Array,
    A_k_cache: jax.Array,
    A_v_cache: jax.Array,
    A_wq: jax.Array,
    A_wo: jax.Array,
    B_x: jax.Array,
    B_w1: jax.Array,
    B_w3: jax.Array,
    B_w2: jax.Array,
    gate_w: jax.Array,
):
    del B_x
    _, _, d_model = A_x.shape
    _, n_heads, seq, dh = A_k_cache.shape
    d_ff = B_w1.shape[1]
    win = min(4096, max(256, seq // 4))

    kt = jnp.swapaxes(A_k_cache, 2, 3)
    vt = jnp.swapaxes(A_v_cache, 2, 3)
    gw = gate_w.reshape(d_model // LANES, LANES)

    kernel = functools.partial(
        _kernel, n_heads=n_heads, dh=dh, seq=seq, win=win, d_model=d_model, d_ff=d_ff)
    return pl.pallas_call(
        kernel,
        out_shape=jax.ShapeDtypeStruct(A_x.shape, A_x.dtype),
        in_specs=[pl.BlockSpec(memory_space=pl.ANY)] * 9,
        out_specs=pl.BlockSpec(memory_space=pltpu.VMEM),
        scratch_shapes=[
            pltpu.VMEM((NSLOT, dh, LANES), jnp.bfloat16),
            pltpu.VMEM(A_x.shape, jnp.bfloat16),
            pltpu.VMEM(gw.shape, jnp.bfloat16),
            pltpu.VMEM((d_model, LANES), jnp.float32),
            pltpu.VMEM((n_heads * dh // LANES, LANES), jnp.float32),
            pltpu.VMEM((d_ff // LANES, LANES), jnp.float32),
            pltpu.VMEM((dh, LANES), jnp.float32),
            pltpu.VMEM((d_ff + n_heads * dh, LANES), jnp.float32),
            pltpu.VMEM((win // LANES, LANES), jnp.float32),
            pltpu.SemaphoreType.DMA((NSLOT + 2,)),
        ],
        compiler_params=pltpu.CompilerParams(
            vmem_limit_bytes=32 * 1024 * 1024,
            disable_bounds_checks=True,
            disable_semaphore_checks=True,
        ),
    )(A_x, kt, vt, A_wq, A_wo, B_w1, B_w3, B_w2, gw)
```

```python
import functools

import jax
import jax.numpy as jnp
from jax import lax
from jax.experimental import pallas as pl
from jax.experimental.pallas import tpu as pltpu

LANES = 128
SUB = 8
HI_ROWS = 16
NQ_STR = 10
NF_STR = 5
NO_STR = 16
N2_STR = 4
P3_RING = 8


def _col_bcast(row):
    n = row.shape[1]
    return jnp.broadcast_to(row, (LANES, n)).T


def _bcast_group(row, off, n):
    lane = lax.broadcasted_iota(jnp.int32, (n, LANES), 1)
    idx = lax.broadcasted_iota(jnp.int32, (n, LANES), 0)
    picked = jnp.where(lane - idx == off, row, 0.0)
    return jnp.broadcast_to(jnp.sum(picked, axis=1, keepdims=True), (n, LANES))


def _tree_sum(parts):
    parts = list(parts)
    while len(parts) > 1:
        nxt = [parts[i] + parts[i + 1] for i in range(0, len(parts) - 1, 2)]
        if len(parts) % 2:
            nxt.append(parts[-1])
        parts = nxt
    return parts[0]


def _fold8(v):
    return _tree_sum(v[i:i + SUB] for i in range(0, v.shape[0], SUB))


def _mult(v, m):
    return v if isinstance(v, int) else pl.multiple_of(v, m)


def _kernel(x_hbm, kt_hbm, vt_hbm, wq_hbm, wo_hbm, w1_hbm, w3_hbm, w2_hbm, gw_hbm,
            out_ref,
            ring1, ring2, ring3, xv, gv, xb_ref, acc_ref, h_ref, qb_ref, cb_ref, s_ref,
            sems,
            *, n_heads, dh, seq, win, d_model, d_ff):
    f32 = jnp.float32
    n_ct = win // LANES
    n_q = (n_heads * dh) // LANES
    n_f = d_ff // LANES
    n_oc = d_model // LANES
    q_rows = d_model // NQ_STR
    f_rows = d_model // NF_STR
    n_r2 = f_rows // SUB
    o_rows = (n_heads * dh) // NO_STR
    n_r3 = o_rows // SUB
    assert f_rows == 2 * q_rows and n_q == 4 * n_f
    assert d_ff == N2_STR * o_rows and o_rows == 2 * dh
    col0 = seq - win
    scale = float(dh) ** -0.5

    ns1, ns2, ns3 = 4 * n_f, 2 * n_ct, P3_RING * n_oc
    sem1, sem2, sem3, sem_x = 0, ns1, ns1 + ns2, ns1 + ns2 + ns3

    def copy(src, dst, sem, prio):
        pltpu.make_async_copy(src, dst, sems.at[sem]).start(priority=prio)

    def wait(buf, sem):
        pltpu.make_async_copy(buf, buf, sems.at[sem]).wait()

    def slot1(r2, c2):
        return (r2 & 3) * n_f + c2

    def start_p1(r2, c2):
        slot = slot1(r2, c2)
        rq = pl.ds(_mult((r2 >> 1) * SUB, SUB), SUB)
        cq = pl.ds(_mult(((r2 & 1) * n_f + c2) * (2 * LANES), 2 * LANES), 2 * LANES)
        rf = pl.ds(_mult(r2 * SUB, SUB), SUB)
        cf = pl.ds(_mult(c2 * LANES, LANES), LANES)
        fs = pl.ds(NQ_STR, NF_STR)
        copy(w1_hbm.at[:, rf, cf], ring1.at[slot, fs, :, pl.ds(0, LANES)], sem1 + slot, 0)
        copy(wq_hbm.at[:, rq, cq], ring1.at[slot, pl.ds(0, NQ_STR)], sem1 + slot, 1)
        copy(w3_hbm.at[:, rf, cf], ring1.at[slot, fs, :, pl.ds(LANES, LANES)], sem1 + slot, 1)

    def start_kv(src, h, c, slot):
        cols = pl.ds(_mult(col0 + c * LANES, LANES), LANES)
        for prio, rows in enumerate((pl.ds(0, HI_ROWS), pl.ds(HI_ROWS, dh - HI_ROWS))):
            copy(src.at[0, h, rows, cols], ring2.at[slot, rows, :], sem2 + slot, prio)

    def slot3(r, c):
        return (r & (P3_RING - 1)) * n_oc + c

    def start_p3(r, c):
        slot = slot3(r, c)
        rows = pl.ds(_mult(r * SUB, SUB), SUB)
        cols = pl.ds(_mult(c * LANES, LANES), LANES)
        copy(w2_hbm.at[:, rows, cols], ring3.at[slot, pl.ds(NO_STR, N2_STR)], sem3 + slot, 0)
        copy(wo_hbm.at[:, rows, cols], ring3.at[slot, pl.ds(0, NO_STR)], sem3 + slot, 1)

    copy(x_hbm, xv, sem_x, 0)
    copy(gw_hbm, gv, sem_x + 1, 0)
    for r2 in range(2):
        for c2 in range(n_f):
            start_p1(r2, c2)

    acc_ref[...] = jnp.zeros(acc_ref.shape, f32)
    wait(xv, sem_x)
    wait(gv, sem_x + 1)
    x = xv[0].astype(f32)
    gw = gv[...].astype(f32)
    gacc = x[:, 0:LANES] * gw[0:1, :]
    for r in range(1, n_oc):
        gacc = gacc + x[:, r * LANES:(r + 1) * LANES] * gw[r:r + 1, :]
    g = jax.nn.sigmoid(jnp.sum(gacc, axis=1, keepdims=True))
    xb_ref[...] = _col_bcast(x)

    def p1_body(r2, carry, *, tail):
        rq = (r2 >> 1) * SUB
        xs = [xb_ref[pl.ds(_mult(i * q_rows + rq, SUB), SUB), :] for i in range(NQ_STR)]
        xs += [xb_ref[pl.ds(_mult(i * f_rows + r2 * SUB, SUB), SUB), :]
               for i in range(NF_STR)]

        def step(c2, carry):
            slot = slot1(r2, c2)
            wait(ring1.at[slot], sem1 + slot)
            if tail:
                c = (r2 - (n_r2 - 2)) * n_f + c2
                start_kv(kt_hbm, 0, c, c)
            else:
                start_p1(r2 + 2, c2)
            t = ring1[slot].astype(f32)
            jq = 2 * ((r2 & 1) * n_f + c2)
            for half in range(2):
                prod = [t[i, :, half * LANES:(half + 1) * LANES] * xs[i]
                        for i in range(NQ_STR + NF_STR)]
                acc_ref[jq + half] += _tree_sum(prod[:NQ_STR])
                acc_ref[n_q + half * n_f + c2] += _tree_sum(prod[NQ_STR:])
            return carry

        return lax.fori_loop(0, n_f, step, carry)

    with jax.named_scope("p1"):
        lax.fori_loop(0, n_r2 - 2, functools.partial(p1_body, tail=False), 0)
        lax.fori_loop(n_r2 - 2, n_r2, functools.partial(p1_body, tail=True), 0)
    for c in range(2 * n_f, n_ct):
        start_kv(kt_hbm, 0, c, c)

    hg = LANES // 2
    h_per = d_ff // n_heads
    assert dh == 3 * hg and h_per == 48 and o_rows % h_per == 0

    def make_qb(h):
        r0 = (3 * h) >> 1
        par = h & 1
        for gi, (r, off) in enumerate(
                ((r0, par * hg), (r0 + par, (1 - par) * hg), (r0 + 1, par * hg))):
            row = jnp.sum(acc_ref[r], axis=0, keepdims=True) * scale
            qb_ref[pl.ds(gi * hg, hg), :] = _bcast_group(row, off, hg)

    def make_hb(h):
        per_str = o_rows // h_per
        for t in range(h_per // 16):
            e = h * h_per + t * 16
            row0 = (h & (per_str - 1)) * h_per + t * 16
            cb_ref[NO_STR + h // per_str, pl.ds(_mult(row0, 16), 16), :] = _bcast_group(
                h_ref[pl.ds(e >> 7, 1), :], e & (LANES - 1), 16)

    make_qb(0)
    for f in range(n_f):
        gate = jnp.sum(acc_ref[n_q + f], axis=0, keepdims=True)
        up = jnp.sum(acc_ref[n_q + n_f + f], axis=0, keepdims=True)
        h_ref[pl.ds(f, 1), :] = (gate * jax.nn.sigmoid(gate)) * up * (1.0 - g)

    def head_body(h, carry, *, last):
        qb = qb_ref[...]

        def k_step(c, carry):
            wait(ring2.at[c], sem2 + c)
            start_kv(vt_hbm, h, c, n_ct + c)
            t = ring2[c].astype(f32)
            s_ref[pl.ds(c, 1), :] = jnp.sum(_fold8(t * qb), axis=0, keepdims=True)
            return carry

        lax.fori_loop(0, n_ct, k_step, 0)

        s = s_ref[...]
        m = jnp.max(jnp.max(s, axis=0, keepdims=True), axis=1, keepdims=True)
        p = jnp.exp(s - m)
        l_row = jnp.sum(p, axis=0, keepdims=True)
        s_ref[...] = p
        if not last:
            make_qb(h + 1)
        make_hb(h)

        def v_step(c, acc):
            wait(ring2.at[n_ct + c], sem2 + n_ct + c)
            if last:
                start_p3(lax.div(c, n_oc), lax.rem(c, n_oc))
            else:
                start_kv(kt_hbm, h + 1, c, c)
            t = ring2[n_ct + c].astype(f32)
            return acc + t * s_ref[pl.ds(c, 1), :]

        acc = lax.fori_loop(0, n_ct, v_step, jnp.zeros((dh, LANES), f32))
        if last:
            for i in range(n_ct, (P3_RING - 1) * n_oc):
                start_p3(i // n_oc, i % n_oc)
        l = jnp.sum(l_row, axis=1, keepdims=True)
        o = jnp.sum(acc, axis=1, keepdims=True) * (g / l)
        cb_ref[h >> 1, pl.ds(_mult((h & 1) * dh, dh), dh), :] = jnp.broadcast_to(
            o, (dh, LANES))
        return carry

    with jax.named_scope("p2"):
        lax.fori_loop(0, n_heads - 1, functools.partial(head_body, last=False), 0)
        head_body(n_heads - 1, 0, last=True)

    def p3_body(r, acc, *, prefetch):
        cb = cb_ref[:, pl.ds(_mult(r * SUB, SUB), SUB), :]
        new = []
        for c in range(n_oc):
            slot = slot3(r, c)
            wait(ring3.at[slot], sem3 + slot)
            if prefetch:
                start_p3(r + P3_RING - 1, c)
            prod = ring3[slot].astype(f32) * cb
            new.append(acc[c] + _tree_sum(prod[i] for i in range(NO_STR + N2_STR)))
        return tuple(new)

    acc = tuple(jnp.zeros((SUB, LANES), f32) for _ in range(n_oc))
    r_hi = n_r3 - (P3_RING - 1)
    with jax.named_scope("p3"):
        acc = lax.fori_loop(0, r_hi, functools.partial(p3_body, prefetch=True), acc)
        acc = lax.fori_loop(r_hi, n_r3, functools.partial(p3_body, prefetch=False), acc)

    res = jnp.concatenate([jnp.sum(a, axis=0, keepdims=True) for a in acc], axis=1)
    out_ref[0] = res.astype(out_ref.dtype)


@jax.jit
def pallas_gated_mix__sliding_block_cached__glu_gated_swiglu__decode_kernel(
    A_x: jax.Array,
    A_k_cache: jax.Array,
    A_v_cache: jax.Array,
    A_wq: jax.Array,
    A_wo: jax.Array,
    B_x: jax.Array,
    B_w1: jax.Array,
    B_w3: jax.Array,
    B_w2: jax.Array,
    gate_w: jax.Array,
):
    del B_x
    _, _, d_model = A_x.shape
    _, n_heads, seq, dh = A_k_cache.shape
    d_ff = B_w1.shape[1]
    win = min(4096, max(256, seq // 4))
    bf16, f32 = jnp.bfloat16, jnp.float32

    def streams(w, n):
        return w.reshape(n, w.shape[0] // n, w.shape[1])

    kt = jnp.swapaxes(A_k_cache, 2, 3)
    vt = jnp.swapaxes(A_v_cache, 2, 3)
    gw = gate_w.reshape(d_model // LANES, LANES)

    n_f = d_ff // LANES
    n_ct = win // LANES
    n_oc = d_model // LANES
    n_q = n_heads * dh // LANES
    n_sems = 4 * n_f + 2 * n_ct + P3_RING * n_oc + 2

    kernel = functools.partial(
        _kernel, n_heads=n_heads, dh=dh, seq=seq, win=win, d_model=d_model, d_ff=d_ff)
    return pl.pallas_call(
        kernel,
        out_shape=jax.ShapeDtypeStruct(A_x.shape, A_x.dtype),
        in_specs=[pl.BlockSpec(memory_space=pl.ANY)] * 9,
        out_specs=pl.BlockSpec(memory_space=pltpu.VMEM),
        scratch_shapes=[
            pltpu.VMEM((4 * n_f, NQ_STR + NF_STR, SUB, 2 * LANES), bf16),
            pltpu.VMEM((2 * n_ct, dh, LANES), bf16),
            pltpu.VMEM((P3_RING * n_oc, NO_STR + N2_STR, SUB, LANES), bf16),
            pltpu.VMEM(A_x.shape, bf16),
            pltpu.VMEM(gw.shape, bf16),
            pltpu.VMEM((d_model, LANES), f32),
            pltpu.VMEM((n_q + 2 * n_f, SUB, LANES), f32),
            pltpu.VMEM((n_f, LANES), f32),
            pltpu.VMEM((dh, LANES), f32),
            pltpu.VMEM((NO_STR + N2_STR, n_heads * dh // NO_STR, LANES), f32),
            pltpu.VMEM((n_ct, LANES), f32),
            pltpu.SemaphoreType.DMA((n_sems,)),
        ],
        compiler_params=pltpu.CompilerParams(
            vmem_limit_bytes=32 * 1024 * 1024,
            disable_bounds_checks=True,
            disable_semaphore_checks=True,
        ),
    )(A_x, kt, vt, streams(A_wq, NQ_STR), streams(A_wo, NO_STR), streams(B_w1, NF_STR),
      streams(B_w3, NF_STR), streams(B_w2, N2_STR), gw)
```

```python
import functools

import jax
import jax.numpy as jnp
from jax import lax
from jax.experimental import pallas as pl
from jax.experimental.pallas import tpu as pltpu

LANES = 128
SUB = 8
HI_ROWS = 16
NQ_STR = 10
NF_STR = 5
NO_STR = 16
N2_STR = 4
P3_RING = 8
P3_AHEAD = 7


def _col_bcast(row):
    n = row.shape[1]
    return jnp.broadcast_to(row, (LANES, n)).T


def _bcast_group(row, off, n):
    lane = lax.broadcasted_iota(jnp.int32, (n, LANES), 1)
    idx = lax.broadcasted_iota(jnp.int32, (n, LANES), 0)
    picked = jnp.where(lane - idx == off, row, 0.0)
    return jnp.broadcast_to(jnp.sum(picked, axis=1, keepdims=True), (n, LANES))


def _tree_sum(parts):
    parts = list(parts)
    while len(parts) > 1:
        nxt = [parts[i] + parts[i + 1] for i in range(0, len(parts) - 1, 2)]
        if len(parts) % 2:
            nxt.append(parts[-1])
        parts = nxt
    return parts[0]


def _fold8(v):
    return _tree_sum(v[i:i + SUB] for i in range(0, v.shape[0], SUB))


def _mult(v, m):
    return v if isinstance(v, int) else pl.multiple_of(v, m)


def _kernel(x_hbm, kt_hbm, vt_hbm, wq_hbm, wo_hbm, w1_hbm, w3_hbm, w2_hbm, gw_hbm,
            out_ref,
            ring1, ring2, ring3, xv, gv, xb_ref, acc_ref, h_ref, qb_ref, cb_ref, s_ref,
            sems,
            *, n_heads, dh, seq, win, d_model, d_ff):
    f32 = jnp.float32
    n_ct = win // LANES
    n_q = (n_heads * dh) // LANES
    n_f = d_ff // LANES
    n_oc = d_model // LANES
    q_rows = d_model // NQ_STR
    f_rows = d_model // NF_STR
    n_r2 = f_rows // SUB
    o_rows = (n_heads * dh) // NO_STR
    n_r3 = o_rows // SUB
    assert f_rows == 2 * q_rows and n_q == 4 * n_f
    assert d_ff == N2_STR * o_rows
    col0 = seq - win
    scale = float(dh) ** -0.5

    ns1, ns2, ns3 = 4 * n_f, 2 * n_ct, P3_RING * n_oc
    sem1, sem2, sem3, sem_x = 0, ns1, ns1 + ns2, ns1 + ns2 + ns3

    def copy(src, dst, sem, prio):
        pltpu.make_async_copy(src, dst, sems.at[sem]).start(priority=prio)

    def wait(buf, sem):
        pltpu.make_async_copy(buf, buf, sems.at[sem]).wait()

    def slot1(r2, c2):
        return (r2 & 3) * n_f + c2

    def start_p1(r2, c2):
        slot = slot1(r2, c2)
        rq = pl.ds(_mult((r2 >> 1) * SUB, SUB), SUB)
        cq = pl.ds(_mult(((r2 & 1) * n_f + c2) * (2 * LANES), 2 * LANES), 2 * LANES)
        rf = pl.ds(_mult(r2 * SUB, SUB), SUB)
        cf = pl.ds(_mult(c2 * LANES, LANES), LANES)
        fs = pl.ds(NQ_STR, NF_STR)
        copy(w1_hbm.at[:, rf, cf], ring1.at[slot, fs, :, pl.ds(0, LANES)], sem1 + slot, 0)
        copy(wq_hbm.at[:, rq, cq], ring1.at[slot, pl.ds(0, NQ_STR)], sem1 + slot, 1)
        copy(w3_hbm.at[:, rf, cf], ring1.at[slot, fs, :, pl.ds(LANES, LANES)], sem1 + slot, 1)

    def start_kv(src, h, c, slot):
        cols = pl.ds(_mult(col0 + c * LANES, LANES), LANES)
        for prio, rows in enumerate((pl.ds(0, HI_ROWS), pl.ds(HI_ROWS, dh - HI_ROWS))):
            copy(src.at[0, h, rows, cols], ring2.at[slot, rows, :], sem2 + slot, prio)

    def slot3(r, c):
        return (r & (P3_RING - 1)) * n_oc + c

    def start_p3(r, c):
        slot = slot3(r, c)
        rows = pl.ds(_mult(r * SUB, SUB), SUB)
        cols = pl.ds(_mult(c * LANES, LANES), LANES)
        copy(w2_hbm.at[:, rows, cols], ring3.at[slot, pl.ds(NO_STR, N2_STR)], sem3 + slot, 0)
        copy(wo_hbm.at[:, rows, cols], ring3.at[slot, pl.ds(0, NO_STR)], sem3 + slot, 1)

    copy(x_hbm, xv, sem_x, 0)
    copy(gw_hbm, gv, sem_x + 1, 0)
    for r2 in range(2):
        for c2 in range(n_f):
            start_p1(r2, c2)

    acc_ref[...] = jnp.zeros(acc_ref.shape, f32)
    wait(xv, sem_x)
    wait(gv, sem_x + 1)
    x = xv[0].astype(f32)
    gw = gv[...].astype(f32)
    gacc = x[:, 0:LANES] * gw[0:1, :]
    for r in range(1, n_oc):
        gacc = gacc + x[:, r * LANES:(r + 1) * LANES] * gw[r:r + 1, :]
    g = jax.nn.sigmoid(jnp.sum(gacc, axis=1, keepdims=True))
    xb_ref[...] = _col_bcast(x)

    def p1_body(r2, carry, *, tail):
        rq = (r2 >> 1) * SUB
        xs = [xb_ref[pl.ds(_mult(i * q_rows + rq, SUB), SUB), :] for i in range(NQ_STR)]
        xs += [xb_ref[pl.ds(_mult(i * f_rows + r2 * SUB, SUB), SUB), :]
               for i in range(NF_STR)]

        def step(c2, carry):
            slot = slot1(r2, c2)
            wait(ring1.at[slot], sem1 + slot)
            if tail:
                c = (r2 - (n_r2 - 2)) * n_f + c2
                start_kv(kt_hbm, 0, c, c)
            else:
                start_p1(r2 + 2, c2)
            t = ring1[slot].astype(f32)
            jq = 2 * ((r2 & 1) * n_f + c2)
            for half in range(2):
                prod = [t[i, :, half * LANES:(half + 1) * LANES] * xs[i]
                        for i in range(NQ_STR + NF_STR)]
                acc_ref[jq + half] += _tree_sum(prod[:NQ_STR])
                acc_ref[n_q + half * n_f + c2] += _tree_sum(prod[NQ_STR:])
            return carry

        return lax.fori_loop(0, n_f, step, carry)

    with jax.named_scope("p1"):
        lax.fori_loop(0, n_r2 - 2, functools.partial(p1_body, tail=False), 0)
        lax.fori_loop(n_r2 - 2, n_r2, functools.partial(p1_body, tail=True), 0)
    for c in range(2 * n_f, n_ct):
        start_kv(kt_hbm, 0, c, c)

    hg = LANES // 2
    h_per = d_ff // n_heads
    assert dh == 3 * hg and h_per % 16 == 0

    def make_qb(h):
        r0 = (3 * h) >> 1
        par = h & 1
        for gi, (r, off) in enumerate(
                ((r0, par * hg), (r0 + par, (1 - par) * hg), (r0 + 1, par * hg))):
            row = jnp.sum(acc_ref[r], axis=0, keepdims=True) * scale
            qb_ref[pl.ds(gi * hg, hg), :] = _bcast_group(row, off, hg)

    def make_hb(h):
        for t in range(h_per // 16):
            e = h * h_per + t * 16
            cb_ref[pl.ds(_mult(n_heads * dh + e, 16), 16), :] = _bcast_group(
                h_ref[pl.ds(e >> 7, 1), :], e & (LANES - 1), 16)

    make_qb(0)
    for f in range(n_f):
        gate = jnp.sum(acc_ref[n_q + f], axis=0, keepdims=True)
        up = jnp.sum(acc_ref[n_q + n_f + f], axis=0, keepdims=True)
        h_ref[pl.ds(f, 1), :] = (gate * jax.nn.sigmoid(gate)) * up * (1.0 - g)

    def head_body(h, carry, *, last):
        qb = qb_ref[...]

        def k_step(c, carry):
            wait(ring2.at[c], sem2 + c)
            start_kv(vt_hbm, h, c, n_ct + c)
            t = ring2[c].astype(f32)
            s_ref[pl.ds(c, 1), :] = jnp.sum(_fold8(t * qb), axis=0, keepdims=True)
            return carry

        lax.fori_loop(0, n_ct, k_step, 0)

        s = s_ref[...]
        m = jnp.max(jnp.max(s, axis=0, keepdims=True), axis=1, keepdims=True)
        p = jnp.exp(s - m)
        l_row = jnp.sum(p, axis=0, keepdims=True)
        s_ref[...] = p
        if not last:
            make_qb(h + 1)
        make_hb(h)

        def v_step(c, acc):
            wait(ring2.at[n_ct + c], sem2 + n_ct + c)
            if last:
                start_p3(lax.div(c, n_oc), lax.rem(c, n_oc))
            else:
                start_kv(kt_hbm, h + 1, c, c)
            t = ring2[n_ct + c].astype(f32)
            return acc + t * s_ref[pl.ds(c, 1), :]

        acc = lax.fori_loop(0, n_ct, v_step, jnp.zeros((dh, LANES), f32))
        if last:
            for i in range(n_ct, P3_AHEAD * n_oc):
                start_p3(i // n_oc, i % n_oc)
        l = jnp.sum(l_row, axis=1, keepdims=True)
        o = jnp.sum(acc, axis=1, keepdims=True) * (g / l)
        cb_ref[pl.ds(_mult(h * dh, dh), dh), :] = jnp.broadcast_to(o, (dh, LANES))
        return carry

    with jax.named_scope("p2"):
        lax.fori_loop(0, n_heads - 1, functools.partial(head_body, last=False), 0)
        head_body(n_heads - 1, 0, last=True)

    def p3_body(r, acc, *, prefetch):
        cb = [cb_ref[pl.ds(_mult(i * o_rows + r * SUB, SUB), SUB), :]
              for i in range(NO_STR + N2_STR)]
        new = []
        for c in range(n_oc):
            slot = slot3(r, c)
            wait(ring3.at[slot], sem3 + slot)
            if prefetch:
                start_p3(r + P3_AHEAD, c)
            t = ring3[slot].astype(f32)
            new.append(acc[c] + _tree_sum(t[i] * cb[i] for i in range(NO_STR + N2_STR)))
        return tuple(new)

    acc = tuple(jnp.zeros((SUB, LANES), f32) for _ in range(n_oc))
    r_hi = n_r3 - P3_AHEAD
    with jax.named_scope("p3"):
        acc = lax.fori_loop(0, r_hi, functools.partial(p3_body, prefetch=True), acc)
        acc = lax.fori_loop(r_hi, n_r3, functools.partial(p3_body, prefetch=False), acc)

    res = jnp.concatenate([jnp.sum(a, axis=0, keepdims=True) for a in acc], axis=1)
    out_ref[0] = res.astype(out_ref.dtype)


@jax.jit
def pallas_gated_mix__sliding_block_cached__glu_gated_swiglu__decode_kernel(
    A_x: jax.Array,
    A_k_cache: jax.Array,
    A_v_cache: jax.Array,
    A_wq: jax.Array,
    A_wo: jax.Array,
    B_x: jax.Array,
    B_w1: jax.Array,
    B_w3: jax.Array,
    B_w2: jax.Array,
    gate_w: jax.Array,
):
    del B_x
    _, _, d_model = A_x.shape
    _, n_heads, seq, dh = A_k_cache.shape
    d_ff = B_w1.shape[1]
    win = min(4096, max(256, seq // 4))
    bf16, f32 = jnp.bfloat16, jnp.float32

    def streams(w, n):
        return w.reshape(n, w.shape[0] // n, w.shape[1])

    kt = jnp.swapaxes(A_k_cache, 2, 3)
    vt = jnp.swapaxes(A_v_cache, 2, 3)
    gw = gate_w.reshape(d_model // LANES, LANES)

    n_f = d_ff // LANES
    n_ct = win // LANES
    n_oc = d_model // LANES
    n_q = n_heads * dh // LANES
    n_sems = 4 * n_f + 2 * n_ct + P3_RING * n_oc + 2

    kernel = functools.partial(
        _kernel, n_heads=n_heads, dh=dh, seq=seq, win=win, d_model=d_model, d_ff=d_ff)
    return pl.pallas_call(
        kernel,
        out_shape=jax.ShapeDtypeStruct(A_x.shape, A_x.dtype),
        in_specs=[pl.BlockSpec(memory_space=pl.ANY)] * 9,
        out_specs=pl.BlockSpec(memory_space=pltpu.VMEM),
        scratch_shapes=[
            pltpu.VMEM((4 * n_f, NQ_STR + NF_STR, SUB, 2 * LANES), bf16),
            pltpu.VMEM((2 * n_ct, dh, LANES), bf16),
            pltpu.VMEM((P3_RING * n_oc, NO_STR + N2_STR, SUB, LANES), bf16),
            pltpu.VMEM(A_x.shape, bf16),
            pltpu.VMEM(gw.shape, bf16),
            pltpu.VMEM((d_model, LANES), f32),
            pltpu.VMEM((n_q + 2 * n_f, SUB, LANES), f32),
            pltpu.VMEM((n_f, LANES), f32),
            pltpu.VMEM((dh, LANES), f32),
            pltpu.VMEM((n_heads * dh + d_ff, LANES), f32),
            pltpu.VMEM((n_ct, LANES), f32),
            pltpu.SemaphoreType.DMA((n_sems,)),
        ],
        compiler_params=pltpu.CompilerParams(
            vmem_limit_bytes=32 * 1024 * 1024,
            disable_bounds_checks=True,
            disable_semaphore_checks=True,
        ),
    )(A_x, kt, vt, streams(A_wq, NQ_STR), streams(A_wo, NO_STR), streams(B_w1, NF_STR),
      streams(B_w3, NF_STR), streams(B_w2, N2_STR), gw)
```

```python
import functools

import jax
import jax.numpy as jnp
from jax import lax
from jax.experimental import pallas as pl
from jax.experimental.pallas import tpu as pltpu

LANES = 128
SUB = 8
HI_ROWS = 24
NB = 15
NS = 4
HI_STR = 2
NSLOT = 64


def _col_bcast(row):
    n = row.shape[1]
    return jnp.broadcast_to(row, (LANES, n)).T


def _bcast_group(row, off, n):
    lane = lax.broadcasted_iota(jnp.int32, (n, LANES), 1)
    idx = lax.broadcasted_iota(jnp.int32, (n, LANES), 0)
    picked = jnp.where(lane - idx == off, row, 0.0)
    return jnp.broadcast_to(jnp.sum(picked, axis=1, keepdims=True), (n, LANES))


def _tree_sum(parts):
    parts = list(parts)
    while len(parts) > 1:
        nxt = [parts[i] + parts[i + 1] for i in range(0, len(parts) - 1, 2)]
        if len(parts) % 2:
            nxt.append(parts[-1])
        parts = nxt
    return parts[0]


def _fold8(v):
    return _tree_sum(v[i:i + SUB] for i in range(0, v.shape[0], SUB))


def _mult(v, m):
    return v if isinstance(v, int) else pl.multiple_of(v, m)


def _rows8(ref, group):
    return ref[pl.ds(_mult(group * SUB, SUB), SUB), :]


def _kernel(x_hbm, kt_hbm, vt_hbm, wq_hbm, wo_hbm, w1_hbm, w3_hbm, w2_hbm, gw_hbm,
            out_ref,
            wring, kvring, xv, gv, xb_ref, acc_ref, h_ref, qb_ref, cb_ref, s_ref,
            sems,
            *, n_heads, dh, seq, win, d_model, d_ff):
    f32 = jnp.float32
    n_ct = win // LANES
    n_q = (n_heads * dh) // LANES
    n_f = d_ff // LANES
    n_oc = d_model // LANES
    tb = wq_hbm.shape[1]
    ts = w1_hbm.shape[1]
    col0 = seq - win
    scale = float(dh) ** -0.5
    assert 2 * n_ct == NSLOT
    sem_w, sem_kv, sem_x = 0, NSLOT, 2 * NSLOT

    def copy(src, dst, sem, prio):
        pltpu.make_async_copy(src, dst, sems.at[sem]).start(priority=prio)

    def wait(buf, sem):
        pltpu.make_async_copy(buf, buf, sems.at[sem]).wait()

    def start_w(p, big, smalls):
        slot = p & (NSLOT - 1)
        sem = sem_w + slot
        if smalls:
            copy(smalls[0].at[:, p], wring.at[slot, pl.ds(NB, NS)], sem, 0)
            copy(big.at[:, p], wring.at[slot, pl.ds(0, NB)], sem, 1)
            for k, small in enumerate(smalls[1:], start=1):
                copy(small.at[:, p], wring.at[slot, pl.ds(NB + k * NS, NS)], sem, 1)
        else:
            for prio, st in enumerate((pl.ds(0, HI_STR), pl.ds(HI_STR, NB - HI_STR))):
                copy(big.at[st, p], wring.at[slot, st], sem, prio)

    def wait_w(p, n_small):
        slot = p & (NSLOT - 1)
        n = NB + n_small * NS
        wait(wring.at[slot, pl.ds(0, n)], sem_w + slot)
        return lambda: wring[slot, pl.ds(0, n)].astype(f32)

    def start_kv(src, h, c, slot):
        cols = pl.ds(_mult(col0 + c * LANES, LANES), LANES)
        for prio, rows in enumerate((pl.ds(0, HI_ROWS), pl.ds(HI_ROWS, dh - HI_ROWS))):
            copy(src.at[0, h, rows, cols], kvring.at[slot, rows, :], sem_kv + slot, prio)

    up_w = (w1_hbm, w3_hbm)
    ahead1 = n_ct
    copy(x_hbm, xv, sem_x, 0)
    copy(gw_hbm, gv, sem_x + 1, 0)
    for p in range(ahead1):
        start_w(p, wq_hbm, up_w)

    acc_ref[...] = jnp.zeros(acc_ref.shape, f32)
    wait(xv, sem_x)
    wait(gv, sem_x + 1)
    x = xv[0].astype(f32)
    gw = gv[...].astype(f32)
    gacc = x[:, 0:LANES] * gw[0:1, :]
    for r in range(1, n_oc):
        gacc = gacc + x[:, r * LANES:(r + 1) * LANES] * gw[r:r + 1, :]
    g = jax.nn.sigmoid(jnp.sum(gacc, axis=1, keepdims=True))
    xb_ref[...] = _col_bcast(x)

    seg_len = tb % n_q
    n_cls = n_q // seg_len
    n_seg = tb // seg_len
    assert n_q % seg_len == 0 and tb % seg_len == 0 and NB % n_cls == 0
    assert ts % seg_len == 0 and ts % n_f == 0 and ahead1 % seg_len == 0
    seg_ahead = ahead1 // seg_len
    seg_small = ts // seg_len

    def p1_seg(seg, carry, *, ffn, nxt):
        xs, cols = [None] * NB, []
        for j in range(n_cls):
            if isinstance(seg, int):
                wrap, blk = divmod(seg + j, n_cls)
            else:
                wrap = lax.div(seg + j, n_cls)
                blk = seg + j - wrap * n_cls
            cols.append(blk * seg_len)
            for m in range(NB // n_cls):
                i = n_cls * m + j
                xs[i] = _rows8(xb_ref, (tb * i) // n_q + wrap)

        def step(u, carry):
            rf, cf = carry
            p = seg * seg_len + u
            load = wait_w(p, 2 if ffn else 0)
            if nxt == "ffn":
                start_w(p + ahead1, wq_hbm, up_w)
            elif nxt == "big":
                start_w(p + ahead1, wq_hbm, ())
            else:
                c = p + ahead1 - tb
                start_kv(kt_hbm, 0, c, c)
            t = load()
            for j in range(n_cls):
                acc_ref[cols[j] + u] += _tree_sum(
                    t[i] * xs[i] for i in range(j, NB, n_cls))
            if ffn:
                xf = [_rows8(xb_ref, i * (ts // n_f) + rf) for i in range(NS)]
                for k in range(2):
                    acc_ref[n_q + k * n_f + cf] += _tree_sum(
                        t[NB + k * NS + i] * xf[i] for i in range(NS))
                last = cf == n_f - 1
                rf = jnp.where(last, rf + 1, rf)
                cf = jnp.where(last, 0, cf + 1)
            return rf, cf

        return lax.fori_loop(0, seg_len, step, carry)

    with jax.named_scope("p1"):
        carry = (jnp.int32(0), jnp.int32(0))
        n_uni = seg_small - seg_ahead
        carry = lax.fori_loop(
            0, n_uni, functools.partial(p1_seg, ffn=True, nxt="ffn"), carry)
        for seg in range(n_uni, n_seg):
            carry = p1_seg(seg, carry, ffn=seg < seg_small,
                           nxt="big" if seg + seg_ahead < n_seg else "kv")

    hg = LANES // 2
    h_per = d_ff // n_heads
    assert dh == 3 * hg and h_per % 16 == 0
    ahead3 = 7 * n_oc
    assert n_ct <= ahead3 < NSLOT

    def make_qb(h):
        r0 = (3 * h) >> 1
        par = h & 1
        for gi, (r, off) in enumerate(
                ((r0, par * hg), (r0 + par, (1 - par) * hg), (r0 + 1, par * hg))):
            row = jnp.sum(acc_ref[r], axis=0, keepdims=True) * scale
            qb_ref[pl.ds(gi * hg, hg), :] = _bcast_group(row, off, hg)

    def make_hb(h):
        for t in range(h_per // 16):
            e = h * h_per + t * 16
            cb_ref[pl.ds(_mult(n_heads * dh + e, 16), 16), :] = _bcast_group(
                h_ref[pl.ds(e >> 7, 1), :], e & (LANES - 1), 16)

    make_qb(0)
    for f in range(n_f):
        gate = jnp.sum(acc_ref[n_q + f], axis=0, keepdims=True)
        up = jnp.sum(acc_ref[n_q + n_f + f], axis=0, keepdims=True)
        h_ref[pl.ds(f, 1), :] = (gate * jax.nn.sigmoid(gate)) * up * (1.0 - g)

    def head_body(h, carry, *, last):
        qb = qb_ref[...]

        def k_step(c, carry):
            wait(kvring.at[c], sem_kv + c)
            start_kv(vt_hbm, h, c, n_ct + c)
            t = kvring[c].astype(f32)
            s_ref[pl.ds(c, 1), :] = jnp.sum(_fold8(t * qb), axis=0, keepdims=True)
            return carry

        lax.fori_loop(0, n_ct, k_step, 0)

        s = s_ref[...]
        m = jnp.max(jnp.max(s, axis=0, keepdims=True), axis=1, keepdims=True)
        p = jnp.exp(s - m)
        l_row = jnp.sum(p, axis=0, keepdims=True)
        s_ref[...] = p
        if not last:
            make_qb(h + 1)
        make_hb(h)

        def v_step(c, acc):
            wait(kvring.at[n_ct + c], sem_kv + n_ct + c)
            if last:
                start_w(c, wo_hbm, (w2_hbm,))
            else:
                start_kv(kt_hbm, h + 1, c, c)
            t = kvring[n_ct + c].astype(f32)
            return acc + t * s_ref[pl.ds(c, 1), :]

        acc = lax.fori_loop(0, n_ct, v_step, jnp.zeros((dh, LANES), f32))
        if last:
            for i in range(n_ct, ahead3):
                start_w(i, wo_hbm, (w2_hbm,))
        l = jnp.sum(l_row, axis=1, keepdims=True)
        o = jnp.sum(acc, axis=1, keepdims=True) * (g / l)
        cb_ref[pl.ds(_mult(h * dh, dh), dh), :] = jnp.broadcast_to(o, (dh, LANES))
        return carry

    with jax.named_scope("p2"):
        lax.fori_loop(0, n_heads - 1, functools.partial(head_body, last=False), 0)
        head_body(n_heads - 1, 0, last=True)

    assert ts % n_oc == 0
    w2_grp0 = (n_heads * dh) // SUB

    def p3_group(a, acc, *, kinds):
        acc = list(acc)
        for b, kind in enumerate(kinds):
            if kind is None:
                continue
            small, nxt = kind
            p = a * n_oc + b
            load = wait_w(p, 1 if small else 0)
            if nxt == "ffn":
                start_w(p + ahead3, wo_hbm, (w2_hbm,))
            elif nxt == "big":
                start_w(p + ahead3, wo_hbm, ())
            t = load()
            terms = [[] for _ in range(n_oc)]
            for i in range(NB):
                grp, col = divmod(tb * i + b, n_oc)
                terms[col].append(t[i] * _rows8(cb_ref, grp + a))
            if small:
                for i in range(NS):
                    terms[b].append(
                        t[NB + i] * _rows8(cb_ref, w2_grp0 + i * (ts // n_oc) + a))
            for col in range(n_oc):
                acc[col] = acc[col] + _tree_sum(terms[col])
        return tuple(acc)

    def p3_kind(p):
        if p >= tb:
            return None
        q = p + ahead3
        return (p < ts, "ffn" if q < ts else "big" if q < tb else None)

    acc = tuple(jnp.zeros((SUB, LANES), f32) for _ in range(n_oc))
    n_grp = -(-tb // n_oc)
    kinds = [tuple(p3_kind(a * n_oc + b) for b in range(n_oc)) for a in range(n_grp)]
    with jax.named_scope("p3"):
        a0 = 0
        while a0 < n_grp:
            a1 = a0 + 1
            while a1 < n_grp and kinds[a1] == kinds[a0]:
                a1 += 1
            body = functools.partial(p3_group, kinds=kinds[a0])
            acc = body(a0, acc) if a1 == a0 + 1 else lax.fori_loop(a0, a1, body, acc)
            a0 = a1

    res = jnp.concatenate([jnp.sum(a, axis=0, keepdims=True) for a in acc], axis=1)
    out_ref[0] = res.astype(out_ref.dtype)


@jax.jit
def pallas_gated_mix__sliding_block_cached__glu_gated_swiglu__decode_kernel(
    A_x: jax.Array,
    A_k_cache: jax.Array,
    A_v_cache: jax.Array,
    A_wq: jax.Array,
    A_wo: jax.Array,
    B_x: jax.Array,
    B_w1: jax.Array,
    B_w3: jax.Array,
    B_w2: jax.Array,
    gate_w: jax.Array,
):
    del B_x
    _, _, d_model = A_x.shape
    _, n_heads, seq, dh = A_k_cache.shape
    d_ff = B_w1.shape[1]
    win = min(4096, max(256, seq // 4))
    bf16, f32 = jnp.bfloat16, jnp.float32

    def tile_streams(w, n):
        r, c = w.shape
        tiles = w.reshape(r // SUB, SUB, c // LANES, LANES).transpose(0, 2, 1, 3)
        return tiles.reshape(n, (r // SUB) * (c // LANES) // n, SUB, LANES)

    kt = jnp.swapaxes(A_k_cache, 2, 3)
    vt = jnp.swapaxes(A_v_cache, 2, 3)
    gw = gate_w.reshape(d_model // LANES, LANES)

    n_f = d_ff // LANES
    n_q = n_heads * dh // LANES

    kernel = functools.partial(
        _kernel, n_heads=n_heads, dh=dh, seq=seq, win=win, d_model=d_model, d_ff=d_ff)
    return pl.pallas_call(
        kernel,
        out_shape=jax.ShapeDtypeStruct(A_x.shape, A_x.dtype),
        in_specs=[pl.BlockSpec(memory_space=pl.ANY)] * 9,
        out_specs=pl.BlockSpec(memory_space=pltpu.VMEM),
        scratch_shapes=[
            pltpu.VMEM((NSLOT, NB + 2 * NS, SUB, LANES), bf16),
            pltpu.VMEM((NSLOT, dh, LANES), bf16),
            pltpu.VMEM(A_x.shape, bf16),
            pltpu.VMEM(gw.shape, bf16),
            pltpu.VMEM((d_model, LANES), f32),
            pltpu.VMEM((n_q + 2 * n_f, SUB, LANES), f32),
            pltpu.VMEM((n_f, LANES), f32),
            pltpu.VMEM((dh, LANES), f32),
            pltpu.VMEM((n_heads * dh + d_ff, LANES), f32),
            pltpu.VMEM((win // LANES, LANES), f32),
            pltpu.SemaphoreType.DMA((2 * NSLOT + 2,)),
        ],
        compiler_params=pltpu.CompilerParams(
            vmem_limit_bytes=32 * 1024 * 1024,
            disable_bounds_checks=True,
            disable_semaphore_checks=True,
        ),
    )(A_x, kt, vt, tile_streams(A_wq, NB), tile_streams(A_wo, NB),
      tile_streams(B_w1, NS), tile_streams(B_w3, NS), tile_streams(B_w2, NS), gw)
```

```python
import functools

import jax
import jax.numpy as jnp
from jax import lax
from jax.experimental import pallas as pl
from jax.experimental.pallas import tpu as pltpu

LANES = 128
SUB = 8
HI_ROWS = 16
NB = 15
NS = 4
HI_STR = 2
NSLOT = 64


def _col_bcast(row):
    n = row.shape[1]
    return jnp.broadcast_to(row, (LANES, n)).T


def _bcast_group(row, off, n):
    lane = lax.broadcasted_iota(jnp.int32, (n, LANES), 1)
    idx = lax.broadcasted_iota(jnp.int32, (n, LANES), 0)
    picked = jnp.where(lane - idx == off, row, 0.0)
    return jnp.broadcast_to(jnp.sum(picked, axis=1, keepdims=True), (n, LANES))


def _tree_sum(parts):
    parts = list(parts)
    while len(parts) > 1:
        nxt = [parts[i] + parts[i + 1] for i in range(0, len(parts) - 1, 2)]
        if len(parts) % 2:
            nxt.append(parts[-1])
        parts = nxt
    return parts[0]


def _fold8(v):
    return _tree_sum(v[i:i + SUB] for i in range(0, v.shape[0], SUB))


def _mult(v, m):
    return v if isinstance(v, int) else pl.multiple_of(v, m)


def _rows8(ref, group):
    return ref[pl.ds(_mult(group * SUB, SUB), SUB), :]


def _kernel(x_hbm, kt_hbm, vt_hbm, wq_hbm, wo_hbm, w1_hbm, w3_hbm, w2_hbm, gw_hbm,
            out_ref,
            wring, kvring, xv, gv, xb_ref, acc_ref, h_ref, qb_ref, cb_ref, s_ref,
            sems,
            *, n_heads, dh, seq, win, d_model, d_ff):
    f32 = jnp.float32
    n_ct = win // LANES
    n_q = (n_heads * dh) // LANES
    n_f = d_ff // LANES
    n_oc = d_model // LANES
    tb = wq_hbm.shape[1]
    ts = w1_hbm.shape[1]
    col0 = seq - win
    scale = float(dh) ** -0.5
    assert 2 * n_ct == NSLOT
    sem_w, sem_kv, sem_x = 0, NSLOT, 2 * NSLOT

    def copy(src, dst, sem, prio):
        pltpu.make_async_copy(src, dst, sems.at[sem]).start(priority=prio)

    def wait(buf, sem):
        pltpu.make_async_copy(buf, buf, sems.at[sem]).wait()

    def start_w(p, big, smalls):
        slot = p & (NSLOT - 1)
        sem = sem_w + slot
        if smalls:
            copy(smalls[0].at[:, p], wring.at[slot, pl.ds(NB, NS)], sem, 0)
            copy(big.at[:, p], wring.at[slot, pl.ds(0, NB)], sem, 1)
            for k, small in enumerate(smalls[1:], start=1):
                copy(small.at[:, p], wring.at[slot, pl.ds(NB + k * NS, NS)], sem, 1)
        else:
            for prio, st in enumerate((pl.ds(0, HI_STR), pl.ds(HI_STR, NB - HI_STR))):
                copy(big.at[st, p], wring.at[slot, st], sem, prio)

    def wait_w(p, n_small):
        slot = p & (NSLOT - 1)
        n = NB + n_small * NS
        wait(wring.at[slot, pl.ds(0, n)], sem_w + slot)
        return lambda: wring[slot, pl.ds(0, n)].astype(f32)

    def start_kv(src, h, c, slot):
        cols = pl.ds(_mult(col0 + c * LANES, LANES), LANES)
        for prio, rows in enumerate((pl.ds(0, HI_ROWS), pl.ds(HI_ROWS, dh - HI_ROWS))):
            copy(src.at[0, h, rows, cols], kvring.at[slot, rows, :], sem_kv + slot, prio)

    up_w = (w1_hbm, w3_hbm)
    ahead1 = n_ct
    copy(x_hbm, xv, sem_x, 0)
    copy(gw_hbm, gv, sem_x + 1, 0)
    for p in range(ahead1):
        start_w(p, wq_hbm, up_w)

    acc_ref[...] = jnp.zeros(acc_ref.shape, f32)
    wait(xv, sem_x)
    wait(gv, sem_x + 1)
    x = xv[0].astype(f32)
    gw = gv[...].astype(f32)
    gacc = x[:, 0:LANES] * gw[0:1, :]
    for r in range(1, n_oc):
        gacc = gacc + x[:, r * LANES:(r + 1) * LANES] * gw[r:r + 1, :]
    g = jax.nn.sigmoid(jnp.sum(gacc, axis=1, keepdims=True))
    xb_ref[...] = _col_bcast(x)

    seg_len = tb % n_q
    n_cls = n_q // seg_len
    n_seg = tb // seg_len
    assert n_q % seg_len == 0 and tb % seg_len == 0 and NB % n_cls == 0
    assert ts % seg_len == 0 and ts % n_f == 0 and ahead1 % seg_len == 0
    seg_ahead = ahead1 // seg_len
    seg_small = ts // seg_len

    def p1_seg(seg, carry, *, ffn, nxt):
        xs, cols = [None] * NB, []
        for j in range(n_cls):
            if isinstance(seg, int):
                wrap, blk = divmod(seg + j, n_cls)
            else:
                wrap = lax.div(seg + j, n_cls)
                blk = seg + j - wrap * n_cls
            cols.append(blk * seg_len)
            for m in range(NB // n_cls):
                i = n_cls * m + j
                xs[i] = _rows8(xb_ref, (tb * i) // n_q + wrap)

        def step(u, carry):
            rf, cf = carry
            p = seg * seg_len + u
            load = wait_w(p, 2 if ffn else 0)
            if nxt == "ffn":
                start_w(p + ahead1, wq_hbm, up_w)
            elif nxt == "big":
                start_w(p + ahead1, wq_hbm, ())
            else:
                c = p + ahead1 - tb
                start_kv(kt_hbm, 0, c, c)
            t = load()
            for j in range(n_cls):
                acc_ref[cols[j] + u] += _tree_sum(
                    t[i] * xs[i] for i in range(j, NB, n_cls))
            if ffn:
                xf = [_rows8(xb_ref, i * (ts // n_f) + rf) for i in range(NS)]
                for k in range(2):
                    acc_ref[n_q + k * n_f + cf] += _tree_sum(
                        t[NB + k * NS + i] * xf[i] for i in range(NS))
                last = cf == n_f - 1
                rf = jnp.where(last, rf + 1, rf)
                cf = jnp.where(last, 0, cf + 1)
            return rf, cf

        return lax.fori_loop(0, seg_len, step, carry)

    with jax.named_scope("p1"):
        carry = (jnp.int32(0), jnp.int32(0))
        n_uni = seg_small - seg_ahead
        carry = lax.fori_loop(
            0, n_uni, functools.partial(p1_seg, ffn=True, nxt="ffn"), carry)
        for seg in range(n_uni, n_seg):
            carry = p1_seg(seg, carry, ffn=seg < seg_small,
                           nxt="big" if seg + seg_ahead < n_seg else "kv")

    hg = LANES // 2
    h_per = d_ff // n_heads
    assert dh == 3 * hg and h_per % 16 == 0
    ahead3 = 7 * n_oc
    assert n_ct <= ahead3 < NSLOT

    def make_qb(h):
        r0 = (3 * h) >> 1
        par = h & 1
        for gi, (r, off) in enumerate(
                ((r0, par * hg), (r0 + par, (1 - par) * hg), (r0 + 1, par * hg))):
            row = jnp.sum(acc_ref[r], axis=0, keepdims=True) * scale
            qb_ref[pl.ds(gi * hg, hg), :] = _bcast_group(row, off, hg)

    def make_hb(h):
        for t in range(h_per // 16):
            e = h * h_per + t * 16
            cb_ref[pl.ds(_mult(n_heads * dh + e, 16), 16), :] = _bcast_group(
                h_ref[pl.ds(e >> 7, 1), :], e & (LANES - 1), 16)

    make_qb(0)
    for f in range(n_f):
        gate = jnp.sum(acc_ref[n_q + f], axis=0, keepdims=True)
        up = jnp.sum(acc_ref[n_q + n_f + f], axis=0, keepdims=True)
        h_ref[pl.ds(f, 1), :] = (gate * jax.nn.sigmoid(gate)) * up * (1.0 - g)

    def head_body(h, carry, *, last):
        qb = qb_ref[...]

        def k_step(c, carry):
            wait(kvring.at[c], sem_kv + c)
            start_kv(vt_hbm, h, c, n_ct + c)
            t = kvring[c].astype(f32)
            s_ref[pl.ds(c, 1), :] = jnp.sum(_fold8(t * qb), axis=0, keepdims=True)
            return carry

        lax.fori_loop(0, n_ct, k_step, 0)

        s = s_ref[...]
        m = jnp.max(jnp.max(s, axis=0, keepdims=True), axis=1, keepdims=True)
        p = jnp.exp(s - m)
        l_row = jnp.sum(p, axis=0, keepdims=True)
        s_ref[...] = p
        if not last:
            make_qb(h + 1)
        make_hb(h)

        def v_step(c, acc):
            wait(kvring.at[n_ct + c], sem_kv + n_ct + c)
            if last:
                start_w(c, wo_hbm, (w2_hbm,))
            else:
                start_kv(kt_hbm, h + 1, c, c)
            t = kvring[n_ct + c].astype(f32)
            return acc + t * s_ref[pl.ds(c, 1), :]

        acc = lax.fori_loop(0, n_ct, v_step, jnp.zeros((dh, LANES), f32))
        if last:
            for i in range(n_ct, ahead3):
                start_w(i, wo_hbm, (w2_hbm,))
        l = jnp.sum(l_row, axis=1, keepdims=True)
        o = jnp.sum(acc, axis=1, keepdims=True) * (g / l)
        cb_ref[pl.ds(_mult(h * dh, dh), dh), :] = jnp.broadcast_to(o, (dh, LANES))
        return carry

    with jax.named_scope("p2"):
        lax.fori_loop(0, n_heads - 1, functools.partial(head_body, last=False), 0)
        head_body(n_heads - 1, 0, last=True)

    assert ts % n_oc == 0
    w2_grp0 = (n_heads * dh) // SUB

    def p3_group(a, acc, *, kinds):
        acc = list(acc)
        for b, kind in enumerate(kinds):
            if kind is None:
                continue
            small, nxt = kind
            p = a * n_oc + b
            load = wait_w(p, 1 if small else 0)
            if nxt == "ffn":
                start_w(p + ahead3, wo_hbm, (w2_hbm,))
            elif nxt == "big":
                start_w(p + ahead3, wo_hbm, ())
            t = load()
            terms = [[] for _ in range(n_oc)]
            for i in range(NB):
                grp, col = divmod(tb * i + b, n_oc)
                terms[col].append(t[i] * _rows8(cb_ref, grp + a))
            if small:
                for i in range(NS):
                    terms[b].append(
                        t[NB + i] * _rows8(cb_ref, w2_grp0 + i * (ts // n_oc) + a))
            for col in range(n_oc):
                acc[col] = acc[col] + _tree_sum(terms[col])
        return tuple(acc)

    def p3_kind(p):
        if p >= tb:
            return None
        q = p + ahead3
        return (p < ts, "ffn" if q < ts else "big" if q < tb else None)

    acc = tuple(jnp.zeros((SUB, LANES), f32) for _ in range(n_oc))
    n_grp = -(-tb // n_oc)
    kinds = [tuple(p3_kind(a * n_oc + b) for b in range(n_oc)) for a in range(n_grp)]
    with jax.named_scope("p3"):
        a0 = 0
        while a0 < n_grp:
            a1 = a0 + 1
            while a1 < n_grp and kinds[a1] == kinds[a0]:
                a1 += 1
            body = functools.partial(p3_group, kinds=kinds[a0])
            acc = body(a0, acc) if a1 == a0 + 1 else lax.fori_loop(a0, a1, body, acc)
            a0 = a1

    res = jnp.concatenate([jnp.sum(a, axis=0, keepdims=True) for a in acc], axis=1)
    out_ref[0] = res.astype(out_ref.dtype)


@jax.jit
def pallas_gated_mix__sliding_block_cached__glu_gated_swiglu__decode_kernel(
    A_x: jax.Array,
    A_k_cache: jax.Array,
    A_v_cache: jax.Array,
    A_wq: jax.Array,
    A_wo: jax.Array,
    B_x: jax.Array,
    B_w1: jax.Array,
    B_w3: jax.Array,
    B_w2: jax.Array,
    gate_w: jax.Array,
):
    del B_x
    _, _, d_model = A_x.shape
    _, n_heads, seq, dh = A_k_cache.shape
    d_ff = B_w1.shape[1]
    win = min(4096, max(256, seq // 4))
    bf16, f32 = jnp.bfloat16, jnp.float32

    def tile_streams(w, n):
        r, c = w.shape
        tiles = w.reshape(r // SUB, SUB, c // LANES, LANES).transpose(0, 2, 1, 3)
        return tiles.reshape(n, (r // SUB) * (c // LANES) // n, SUB, LANES)

    kt = jnp.swapaxes(A_k_cache, 2, 3)
    vt = jnp.swapaxes(A_v_cache, 2, 3)
    gw = gate_w.reshape(d_model // LANES, LANES)

    n_f = d_ff // LANES
    n_q = n_heads * dh // LANES

    params = dict(vmem_limit_bytes=32 * 1024 * 1024, disable_bounds_checks=True)
    if hasattr(pltpu.CompilerParams, "disable_semaphore_checks"):
        params["disable_semaphore_checks"] = True

    kernel = functools.partial(
        _kernel, n_heads=n_heads, dh=dh, seq=seq, win=win, d_model=d_model, d_ff=d_ff)
    return pl.pallas_call(
        kernel,
        out_shape=jax.ShapeDtypeStruct(A_x.shape, A_x.dtype),
        in_specs=[pl.BlockSpec(memory_space=pl.ANY)] * 9,
        out_specs=pl.BlockSpec(memory_space=pltpu.VMEM),
        scratch_shapes=[
            pltpu.VMEM((NSLOT, NB + 2 * NS, SUB, LANES), bf16),
            pltpu.VMEM((NSLOT, dh, LANES), bf16),
            pltpu.VMEM(A_x.shape, bf16),
            pltpu.VMEM(gw.shape, bf16),
            pltpu.VMEM((d_model, LANES), f32),
            pltpu.VMEM((n_q + 2 * n_f, SUB, LANES), f32),
            pltpu.VMEM((n_f, LANES), f32),
            pltpu.VMEM((dh, LANES), f32),
            pltpu.VMEM((n_heads * dh + d_ff, LANES), f32),
            pltpu.VMEM((win // LANES, LANES), f32),
            pltpu.SemaphoreType.DMA((2 * NSLOT + 2,)),
        ],
        compiler_params=pltpu.CompilerParams(**params),
    )(A_x, kt, vt, tile_streams(A_wq, NB), tile_streams(A_wo, NB),
      tile_streams(B_w1, NS), tile_streams(B_w3, NS), tile_streams(B_w2, NS), gw)
```

```python
import functools

import jax
import jax.numpy as jnp
from jax import lax
from jax.experimental import pallas as pl
from jax.experimental.pallas import tpu as pltpu

LANES = 128
SUB = 8
HI_ROWS = 16
NB = 15
NS = 4
HI_STR = 2
NSLOT = 64


def _col_bcast(row):
    n = row.shape[1]
    return jnp.broadcast_to(row, (LANES, n)).T


def _bcast_group(row, off, n):
    lane = lax.broadcasted_iota(jnp.int32, (n, LANES), 1)
    idx = lax.broadcasted_iota(jnp.int32, (n, LANES), 0)
    picked = jnp.where(lane - idx == off, row, 0.0)
    return jnp.broadcast_to(jnp.sum(picked, axis=1, keepdims=True), (n, LANES))


def _tree_sum(parts):
    parts = list(parts)
    while len(parts) > 1:
        nxt = [parts[i] + parts[i + 1] for i in range(0, len(parts) - 1, 2)]
        if len(parts) % 2:
            nxt.append(parts[-1])
        parts = nxt
    return parts[0]


def _fold8(v):
    return _tree_sum(v[i:i + SUB] for i in range(0, v.shape[0], SUB))


def _round_bf16(v):
    return v.astype(jnp.bfloat16).astype(jnp.float32)


def _mult(v, m):
    return v if isinstance(v, int) else pl.multiple_of(v, m)


def _rows8(ref, group):
    return ref[pl.ds(_mult(group * SUB, SUB), SUB), :]


def _kernel(x_hbm, kt_hbm, vt_hbm, wq_hbm, wo_hbm, w1_hbm, w3_hbm, w2_hbm, gw_hbm,
            out_ref,
            wring, kvring, xv, gv, xb_ref, acc_ref, h_ref, qb_ref, cb_ref, s_ref,
            sems,
            *, n_heads, dh, seq, win, d_model, d_ff):
    f32 = jnp.float32
    n_ct = win // LANES
    n_q = (n_heads * dh) // LANES
    n_f = d_ff // LANES
    n_oc = d_model // LANES
    tb = wq_hbm.shape[1]
    ts = w1_hbm.shape[1]
    col0 = seq - win
    scale = float(dh) ** -0.5
    assert 2 * n_ct == NSLOT
    sem_w, sem_kv, sem_x = 0, NSLOT, 2 * NSLOT

    def copy(src, dst, sem, prio):
        pltpu.make_async_copy(src, dst, sems.at[sem]).start(priority=prio)

    def wait(buf, sem):
        pltpu.make_async_copy(buf, buf, sems.at[sem]).wait()

    def start_w(p, big, smalls):
        slot = p & (NSLOT - 1)
        sem = sem_w + slot
        if smalls:
            copy(smalls[0].at[:, p], wring.at[slot, pl.ds(NB, NS)], sem, 0)
            copy(big.at[:, p], wring.at[slot, pl.ds(0, NB)], sem, 1)
            for k, small in enumerate(smalls[1:], start=1):
                copy(small.at[:, p], wring.at[slot, pl.ds(NB + k * NS, NS)], sem, 1)
        else:
            for prio, st in enumerate((pl.ds(0, HI_STR), pl.ds(HI_STR, NB - HI_STR))):
                copy(big.at[st, p], wring.at[slot, st], sem, prio)

    def wait_w(p, n_small):
        slot = p & (NSLOT - 1)
        n = NB + n_small * NS
        wait(wring.at[slot, pl.ds(0, n)], sem_w + slot)
        return lambda: wring[slot, pl.ds(0, n)].astype(f32)

    def start_kv(src, h, c, slot):
        cols = pl.ds(_mult(col0 + c * LANES, LANES), LANES)
        for prio, rows in enumerate((pl.ds(0, HI_ROWS), pl.ds(HI_ROWS, dh - HI_ROWS))):
            copy(src.at[0, h, rows, cols], kvring.at[slot, rows, :], sem_kv + slot, prio)

    up_w = (w1_hbm, w3_hbm)
    ahead1 = n_ct
    copy(x_hbm, xv, sem_x, 0)
    copy(gw_hbm, gv, sem_x + 1, 0)
    for p in range(ahead1):
        start_w(p, wq_hbm, up_w)

    acc_ref[...] = jnp.zeros(acc_ref.shape, f32)
    wait(xv, sem_x)
    wait(gv, sem_x + 1)
    x = xv[0].astype(f32)
    gw = gv[...].astype(f32)
    gacc = _tree_sum(_round_bf16(x[:, r * LANES:(r + 1) * LANES] * gw[r:r + 1, :])
                     for r in range(n_oc))
    logit = _round_bf16(jnp.sum(gacc, axis=1, keepdims=True))
    g = _round_bf16(1.0 / _round_bf16(1.0 + _round_bf16(jnp.exp(-logit))))
    g_c = _round_bf16(1.0 - g)
    xb_ref[...] = _col_bcast(x)

    seg_len = tb % n_q
    n_cls = n_q // seg_len
    n_seg = tb // seg_len
    assert n_q % seg_len == 0 and tb % seg_len == 0 and NB % n_cls == 0
    assert ts % seg_len == 0 and ts % n_f == 0 and ahead1 % seg_len == 0
    seg_ahead = ahead1 // seg_len
    seg_small = ts // seg_len

    def p1_seg(seg, carry, *, ffn, nxt):
        xs, cols = [None] * NB, []
        for j in range(n_cls):
            if isinstance(seg, int):
                wrap, blk = divmod(seg + j, n_cls)
            else:
                wrap = lax.div(seg + j, n_cls)
                blk = seg + j - wrap * n_cls
            cols.append(blk * seg_len)
            for m in range(NB // n_cls):
                i = n_cls * m + j
                xs[i] = _rows8(xb_ref, (tb * i) // n_q + wrap)

        def step(u, carry):
            rf, cf = carry
            p = seg * seg_len + u
            load = wait_w(p, 2 if ffn else 0)
            if nxt == "ffn":
                start_w(p + ahead1, wq_hbm, up_w)
            elif nxt == "big":
                start_w(p + ahead1, wq_hbm, ())
            else:
                c = p + ahead1 - tb
                start_kv(kt_hbm, 0, c, c)
            t = load()
            for j in range(n_cls):
                acc_ref[cols[j] + u] += _tree_sum(
                    t[i] * xs[i] for i in range(j, NB, n_cls))
            if ffn:
                xf = [_rows8(xb_ref, i * (ts // n_f) + rf) for i in range(NS)]
                for k in range(2):
                    acc_ref[n_q + k * n_f + cf] += _tree_sum(
                        t[NB + k * NS + i] * xf[i] for i in range(NS))
                last = cf == n_f - 1
                rf = jnp.where(last, rf + 1, rf)
                cf = jnp.where(last, 0, cf + 1)
            return rf, cf

        return lax.fori_loop(0, seg_len, step, carry)

    with jax.named_scope("p1"):
        carry = (jnp.int32(0), jnp.int32(0))
        n_uni = seg_small - seg_ahead
        carry = lax.fori_loop(
            0, n_uni, functools.partial(p1_seg, ffn=True, nxt="ffn"), carry)
        for seg in range(n_uni, n_seg):
            carry = p1_seg(seg, carry, ffn=seg < seg_small,
                           nxt="big" if seg + seg_ahead < n_seg else "kv")

    hg = LANES // 2
    h_per = d_ff // n_heads
    assert dh == 3 * hg and h_per % 16 == 0
    ahead3 = 7 * n_oc
    assert n_ct <= ahead3 < NSLOT

    def make_qb(h):
        r0 = (3 * h) >> 1
        par = h & 1
        for gi, (r, off) in enumerate(
                ((r0, par * hg), (r0 + par, (1 - par) * hg), (r0 + 1, par * hg))):
            row = jnp.sum(acc_ref[r], axis=0, keepdims=True) * scale
            qb_ref[pl.ds(gi * hg, hg), :] = _bcast_group(row, off, hg)

    def make_hb(h):
        for t in range(h_per // 16):
            e = h * h_per + t * 16
            cb_ref[pl.ds(_mult(n_heads * dh + e, 16), 16), :] = _bcast_group(
                h_ref[pl.ds(e >> 7, 1), :], e & (LANES - 1), 16)

    make_qb(0)
    for f in range(n_f):
        gate = jnp.sum(acc_ref[n_q + f], axis=0, keepdims=True)
        up = jnp.sum(acc_ref[n_q + n_f + f], axis=0, keepdims=True)
        h_ref[pl.ds(f, 1), :] = (gate * jax.nn.sigmoid(gate)) * up * g_c

    def head_body(h, carry, *, last):
        qb = qb_ref[...]

        def k_step(c, carry):
            wait(kvring.at[c], sem_kv + c)
            start_kv(vt_hbm, h, c, n_ct + c)
            t = kvring[c].astype(f32)
            s_ref[pl.ds(c, 1), :] = jnp.sum(_fold8(t * qb), axis=0, keepdims=True)
            return carry

        lax.fori_loop(0, n_ct, k_step, 0)

        s = s_ref[...]
        m = jnp.max(jnp.max(s, axis=0, keepdims=True), axis=1, keepdims=True)
        p = jnp.exp(s - m)
        l_row = jnp.sum(p, axis=0, keepdims=True)
        s_ref[...] = p
        if not last:
            make_qb(h + 1)
        make_hb(h)

        def v_step(c, acc):
            wait(kvring.at[n_ct + c], sem_kv + n_ct + c)
            if last:
                start_w(c, wo_hbm, (w2_hbm,))
            else:
                start_kv(kt_hbm, h + 1, c, c)
            t = kvring[n_ct + c].astype(f32)
            return acc + t * s_ref[pl.ds(c, 1), :]

        acc = lax.fori_loop(0, n_ct, v_step, jnp.zeros((dh, LANES), f32))
        if last:
            for i in range(n_ct, ahead3):
                start_w(i, wo_hbm, (w2_hbm,))
        l = jnp.sum(l_row, axis=1, keepdims=True)
        o = jnp.sum(acc, axis=1, keepdims=True) * (g / l)
        cb_ref[pl.ds(_mult(h * dh, dh), dh), :] = jnp.broadcast_to(o, (dh, LANES))
        return carry

    with jax.named_scope("p2"):
        lax.fori_loop(0, n_heads - 1, functools.partial(head_body, last=False), 0)
        head_body(n_heads - 1, 0, last=True)

    assert ts % n_oc == 0
    w2_grp0 = (n_heads * dh) // SUB

    def p3_group(a, acc, *, kinds):
        acc = list(acc)
        for b, kind in enumerate(kinds):
            if kind is None:
                continue
            small, nxt = kind
            p = a * n_oc + b
            load = wait_w(p, 1 if small else 0)
            if nxt == "ffn":
                start_w(p + ahead3, wo_hbm, (w2_hbm,))
            elif nxt == "big":
                start_w(p + ahead3, wo_hbm, ())
            t = load()
            terms = [[] for _ in range(n_oc)]
            for i in range(NB):
                grp, col = divmod(tb * i + b, n_oc)
                terms[col].append(t[i] * _rows8(cb_ref, grp + a))
            if small:
                for i in range(NS):
                    terms[b].append(
                        t[NB + i] * _rows8(cb_ref, w2_grp0 + i * (ts // n_oc) + a))
            for col in range(n_oc):
                acc[col] = acc[col] + _tree_sum(terms[col])
        return tuple(acc)

    def p3_kind(p):
        if p >= tb:
            return None
        q = p + ahead3
        return (p < ts, "ffn" if q < ts else "big" if q < tb else None)

    acc = tuple(jnp.zeros((SUB, LANES), f32) for _ in range(n_oc))
    n_grp = -(-tb // n_oc)
    kinds = [tuple(p3_kind(a * n_oc + b) for b in range(n_oc)) for a in range(n_grp)]
    with jax.named_scope("p3"):
        a0 = 0
        while a0 < n_grp:
            a1 = a0 + 1
            while a1 < n_grp and kinds[a1] == kinds[a0]:
                a1 += 1
            body = functools.partial(p3_group, kinds=kinds[a0])
            acc = body(a0, acc) if a1 == a0 + 1 else lax.fori_loop(a0, a1, body, acc)
            a0 = a1

    res = jnp.concatenate([jnp.sum(a, axis=0, keepdims=True) for a in acc], axis=1)
    out_ref[0] = res.astype(out_ref.dtype)


@jax.jit
def pallas_gated_mix__sliding_block_cached__glu_gated_swiglu__decode_kernel(
    A_x: jax.Array,
    A_k_cache: jax.Array,
    A_v_cache: jax.Array,
    A_wq: jax.Array,
    A_wo: jax.Array,
    B_x: jax.Array,
    B_w1: jax.Array,
    B_w3: jax.Array,
    B_w2: jax.Array,
    gate_w: jax.Array,
):
    del B_x
    _, _, d_model = A_x.shape
    _, n_heads, seq, dh = A_k_cache.shape
    d_ff = B_w1.shape[1]
    win = min(4096, max(256, seq // 4))
    bf16, f32 = jnp.bfloat16, jnp.float32

    def tile_streams(w, n):
        r, c = w.shape
        tiles = w.reshape(r // SUB, SUB, c // LANES, LANES).transpose(0, 2, 1, 3)
        return tiles.reshape(n, (r // SUB) * (c // LANES) // n, SUB, LANES)

    kt = jnp.swapaxes(A_k_cache, 2, 3)
    vt = jnp.swapaxes(A_v_cache, 2, 3)
    gw = gate_w.reshape(d_model // LANES, LANES)

    n_f = d_ff // LANES
    n_q = n_heads * dh // LANES

    params = dict(vmem_limit_bytes=32 * 1024 * 1024, disable_bounds_checks=True)
    if hasattr(pltpu.CompilerParams, "disable_semaphore_checks"):
        params["disable_semaphore_checks"] = True

    kernel = functools.partial(
        _kernel, n_heads=n_heads, dh=dh, seq=seq, win=win, d_model=d_model, d_ff=d_ff)
    return pl.pallas_call(
        kernel,
        out_shape=jax.ShapeDtypeStruct(A_x.shape, A_x.dtype),
        in_specs=[pl.BlockSpec(memory_space=pl.ANY)] * 9,
        out_specs=pl.BlockSpec(memory_space=pltpu.VMEM),
        scratch_shapes=[
            pltpu.VMEM((NSLOT, NB + 2 * NS, SUB, LANES), bf16),
            pltpu.VMEM((NSLOT, dh, LANES), bf16),
            pltpu.VMEM(A_x.shape, bf16),
            pltpu.VMEM(gw.shape, bf16),
            pltpu.VMEM((d_model, LANES), f32),
            pltpu.VMEM((n_q + 2 * n_f, SUB, LANES), f32),
            pltpu.VMEM((n_f, LANES), f32),
            pltpu.VMEM((dh, LANES), f32),
            pltpu.VMEM((n_heads * dh + d_ff, LANES), f32),
            pltpu.VMEM((win // LANES, LANES), f32),
            pltpu.SemaphoreType.DMA((2 * NSLOT + 2,)),
        ],
        compiler_params=pltpu.CompilerParams(**params),
    )(A_x, kt, vt, tile_streams(A_wq, NB), tile_streams(A_wo, NB),
      tile_streams(B_w1, NS), tile_streams(B_w3, NS), tile_streams(B_w2, NS), gw)
```
